```python
import os as _os
_os.environ.setdefault('JAX_PLATFORMS', 'cpu')
import jax
import jax.numpy as jnp

def _softmax(x, axis=-1):
    return jax.nn.softmax(x, axis=axis)

def _gelu(x):
    return jax.nn.gelu(x, approximate=True)

def _silu(x):
    return jax.nn.silu(x)

def _sigmoid(x):
    return jax.nn.sigmoid(x)

def _layernorm(x, axis=-1, eps=1e-05):
    m = jnp.mean(x, axis=axis, keepdims=True)
    v = jnp.var(x, axis=axis, keepdims=True)
    return (x - m) / jnp.sqrt(v + eps)

def _scatter_add(tgt, idx, src, axis=0):
    return tgt.at[idx].add(src)

def _segment_sum(src, seg, n):
    return jax.ops.segment_sum(src, seg, n)

class _Rng:

    def __init__(self, key):
        self._k = key

    def _next(self):
        self._k, sub = jax.random.split(self._k)
        return sub

    def normal(self, shape):
        return jax.random.normal(self._next(), shape, dtype=jnp.bfloat16)

    def randint(self, lo, hi, shape):
        return jax.random.randint(self._next(), shape, lo, hi, dtype=jnp.int32)

    def uniform(self, shape, lo=0.0, hi=1.0):
        return jax.random.uniform(self._next(), shape, jnp.bfloat16, lo, hi)

    def permutation(self, n):
        return jax.random.permutation(self._next(), n)
kernel_name = 'gated_mix__ssm_conv_h3__memory_aug_recurrent_mem_tr__prompt'

def setup_inputs():
    _rng = _Rng(jax.random.key(int.from_bytes(__import__("os").urandom(4), "little")))
    _w = lambda a: (lambda t: t.astype(jnp.bfloat16) if jnp.issubdtype(t.dtype, jnp.floating) else t)(jnp.asarray(a))

    def _A_setup():
        B, S, D = (1, 2048, 1024)
        ks = 4
        return {'q': _w((lambda *s: _rng.normal(s) * 0.05)(B, S, D)), 'k': _w((lambda *s: _rng.normal(s) * 0.4)(B, S, D)), 'v': _w((lambda *s: _rng.normal(s) * 0.4)(B, S, D)), 'shift_k': _w((lambda *s: _rng.normal(s) * 0.4)(D, ks) * 0.5), 'ssm_k': _w((lambda *s: _rng.normal(s) * 0.4)(D, S) * (1.0 / S ** 0.5)), 'ssm_D': _w((lambda *s: _rng.normal(s) * 0.4)(D))}
    _A_in = _A_setup()

    def _B_setup():
        B, S, Dm = (1, 2048, 1024)
        H, Dh = (32, 128)
        M, seg = (8, 32)
        seg = min(seg, S)
        S = S // seg * seg
        return {'x': _w((lambda *s: _rng.normal(s) * 0.05)(B, S, Dm)), 'mem0': _w((lambda *s: _rng.normal(s) * 0.4)(B, M, Dm)), 'Wq': _w((lambda *s: _rng.normal(s) * 3.2)(Dm, H, Dh) * Dm ** (-0.5)), 'Wk': _w((lambda *s: _rng.normal(s) * 3.2)(Dm, H, Dh) * Dm ** (-0.5)), 'Wv': _w((lambda *s: _rng.normal(s) * 0.4)(Dm, H, Dh) * Dm ** (-0.5)), 'Wo': _w((lambda *s: _rng.normal(s) * 0.4)(H, Dh, Dm) * (H * Dh) ** (-0.5)), 'seg_len': seg}
    _B_in = _B_setup()
    return {'A_q': _A_in['q'], 'A_k': _A_in['k'], 'A_v': _A_in['v'], 'A_shift_k': _A_in['shift_k'], 'A_ssm_k': _A_in['ssm_k'], 'A_ssm_D': _A_in['ssm_D'], 'B_x': _B_in['x'], 'B_mem0': _B_in['mem0'], 'B_Wq': _B_in['Wq'], 'B_Wk': _B_in['Wk'], 'B_Wv': _B_in['Wv'], 'B_Wo': _B_in['Wo'], 'B_seg_len': _B_in['seg_len'], 'gate_w': _w((lambda *s: _rng.normal(s) * 0.05)(1024) * 16.0)}

def reference(A_q, A_k, A_v, A_shift_k, A_ssm_k, A_ssm_D, B_x, B_mem0, B_Wq, B_Wk, B_Wv, B_Wo, B_seg_len, gate_w):

    def _A_ref(q, k, v, shift_k, ssm_k, ssm_D):
        B, S, D = q.shape
        ks = shift_k.shape[-1]
        k_pad = jnp.pad(k, ((0, 0), (ks - 1, 0), (0, 0)))
        k_shift = jnp.zeros_like(k)
        for t in range(ks):
            k_shift = k_shift + k_pad[:, t:t + S, :] * shift_k[:, ks - 1 - t][None, None, :]
        kv = k_shift * v
        L = 2 * S
        kv_pad = jnp.pad(kv, ((0, 0), (0, S), (0, 0)))
        kf_pad = jnp.pad(ssm_k, ((0, 0), (0, S)))
        kv_f = (lambda x, axes=(-2, -1): jnp.fft.rfft2(x.astype(jnp.float32), axes=axes))(kv_pad[:, None, :, :], axes=(1, 2))
        kf_f = (lambda x, axes=(-2, -1): jnp.fft.rfft2(x.astype(jnp.float32), axes=axes))(kf_pad[:, None, :], axes=(1, 2))
        kf_f = (lambda x, *d: x.transpose(*d))(kf_f, 1, 2, 0)
        y_f = kv_f * kf_f[None, :, :, :]
        y = (lambda x, s, axes=(-2, -1): jnp.fft.irfft2(x, s=s, axes=axes).astype(jnp.bfloat16))(y_f, (1, L), axes=(1, 2))[:, 0, :S, :]
        y = y + kv * ssm_D[None, None, :]
        return q * y

    def _B_ref(x, mem0, Wq, Wk, Wv, Wo, seg_len):
        B, S, Dm = x.shape
        H, Dh = (Wq.shape[1], Wq.shape[2])
        M = mem0.shape[1]
        scale = Dh ** (-0.5)
        n_seg = S // seg_len
        L = M + seg_len
        idx = jnp.arange(L)
        mask = (idx[:, None] < M) | (idx[:, None] >= idx[None, :])
        mem = mem0
        outs = []
        for s in range(n_seg):
            xs = x[:, s * seg_len:(s + 1) * seg_len, :].copy()
            h = jnp.concatenate([mem, xs], axis=1)
            q = jnp.einsum('btd,dhe->bhte', h, Wq)
            k = jnp.einsum('btd,dhe->bhte', h, Wk)
            v = jnp.einsum('btd,dhe->bhte', h, Wv)
            scores = jnp.einsum('bhqe,bhke->bhqk', q, k) * scale
            scores = jnp.where(mask[None, None], scores, -1000000000.0)
            p = _softmax(scores, axis=-1)
            o = jnp.einsum('bhqk,bhke->bhqe', p, v)
            o = jnp.einsum('bhte,hed->btd', o, Wo)
            mem = o[:, :M, :].copy()
            outs.append(o[:, M:, :])
        return jnp.concatenate(outs, axis=1)
    x = A_q
    g = _sigmoid((x * gate_w).sum(-1, keepdims=True))
    a = _A_ref(x, A_k, A_v, A_shift_k, A_ssm_k, A_ssm_D)
    b = _B_ref(x, B_mem0, B_Wq, B_Wk, B_Wv, B_Wo, B_seg_len)
    return g * a + (1 - g) * b
```

```python
import functools
import math

import jax
import jax.numpy as jnp
from jax import lax
import jax.experimental.pallas as pl
import jax.experimental.pallas.tpu as pltpu

bf16 = jnp.bfloat16
f32 = jnp.float32
u32 = jnp.uint32

S = 2048
D = 1024
H = 32
DH = 128
M = 8
SEG = 32
NSEG = S // SEG
KS = 4
TP = 24
BULK = S - TP * NSEG
RING = 576
NC = D // 128
BL = 128
NB = S // BL
NF = 2 * BL
G = 4
NG = H // G
HC = 8
NCH = 3 * H // HC
PAD = 16
LTOT = SEG + M


def _ring(x):
    x = jnp.where(x >= 2 * RING, x - 2 * RING, x)
    return jnp.where(x >= RING, x - RING, x)


def _kernel(x_hbm, k_hbm, v_hbm, shift_hbm, filt_hbm, dvec_hbm, mem0_hbm,
            wq_hbm, wk_hbm, wv_hbm, wo_hbm, gate_hbm,
            out_hbm,
            x_s, k_s, v_s, f_s, kv_s, a_s, b_s, g_s,
            w_s, wo_s, stage, tmpu, qkv_s, o_s,
            u_s, kf_s, z_s, fw_s, fi_s,
            mem_s, shift_s, dvec_s, gate_s, prm_s, gw_s,
            sem_w, sem_x0, sem_sm, sem_pre, sem_late, sem_out):
    scale = DH ** (-0.5)
    w_hbms = (wq_hbm, wk_hbm, wv_hbm)

    def x0_copy(n):
        return pltpu.make_async_copy(
            x_hbm.at[pl.ds(0, BULK), pl.ds(n * 128, 128)],
            x_s.at[n, pl.ds(0, BULK), :], sem_x0.at[n])

    def w_copy(m, g, slot):
        return pltpu.make_async_copy(
            w_hbms[m].at[:, pl.ds(g * HC, HC), :], stage.at[slot], sem_w.at[slot])

    small = [
        pltpu.make_async_copy(mem0_hbm, mem_s, sem_sm.at[0]),
        pltpu.make_async_copy(shift_hbm, shift_s, sem_sm.at[1]),
        pltpu.make_async_copy(dvec_hbm, dvec_s, sem_sm.at[2]),
        pltpu.make_async_copy(gate_hbm, gate_s, sem_sm.at[3]),
    ]

    def kv_copies(n, sem, base):
        return [
            pltpu.make_async_copy(k_hbm.at[:, pl.ds(n * 128, 128)],
                                  k_s.at[n, pl.ds(PAD, S), :], sem.at[base]),
            pltpu.make_async_copy(v_hbm.at[:, pl.ds(n * 128, 128)],
                                  v_s.at[n], sem.at[base + 1]),
        ]

    pre_groups = []
    idx = 0
    grp = []
    for d in range(NB):
        grp.append(pltpu.make_async_copy(filt_hbm.at[:, pl.ds(d * 128, 128)],
                                         f_s.at[d], sem_pre.at[idx]))
        idx += 1
        if d % 8 == 7:
            pre_groups.append(grp)
            grp = []
    grp = kv_copies(0, sem_pre, idx) + kv_copies(1, sem_pre, idx + 2)
    idx += 4
    pre_groups.append(grp)
    for half in range(2):
        grp = []
        for n in range(half * 4, half * 4 + 4):
            grp.append(pltpu.make_async_copy(
                x_hbm.at[pl.ds(BULK, S - BULK), pl.ds(n * 128, 128)],
                x_s.at[n, pl.ds(BULK, S - BULK), :], sem_pre.at[idx]))
            idx += 1
        pre_groups.append(grp)
    for q in range(4):
        grp = []
        for n in range(2 * q, 2 * q + 2):
            grp.append(pltpu.make_async_copy(wo_hbm.at[:, pl.ds(n * 128, 128)],
                                             wo_s.at[n], sem_pre.at[idx]))
            idx += 1
        pre_groups.append(grp)
    late = []
    for n in range(2, NC):
        late += kv_copies(n, sem_late, 2 * (n - 2))

    def out_copy(n):
        return pltpu.make_async_copy(b_s.at[n], out_hbm.at[:, pl.ds(n * 128, 128)],
                                     sem_out.at[n])

    for n in range(NC):
        x0_copy(n).start()
    w_copy(0, 0, 0).start()
    for c in small:
        c.start()
    w_copy(0, 1, 1).start()
    w_copy(0, 2, 2).start()

    def dft_table(shape, rho_axis):
        rho = lax.broadcasted_iota(jnp.int32, shape, rho_axis)
        t = lax.broadcasted_iota(jnp.int32, shape, 1 - rho_axis)
        f = ((rho >> 5) << 4) + ((rho & 7) << 1) + ((rho >> 3) & 1)
        im = (rho >> 4) & 1
        ph = ((2 * f + 1) * t + im * (BL)) & (4 * BL - 1)
        ph = jnp.where(ph > 2 * BL, 4 * BL - ph, ph)
        return jnp.cos(ph.astype(f32) * (math.pi / NF))

    fw_s[...] = dft_table((NF, BL), 0).astype(bf16)
    fi_s[...] = (dft_table((BL, NF), 1) * (1.0 / BL)).astype(bf16)
    for n in range(NC):
        k_s[n, 0:PAD, :] = jnp.zeros((PAD, 128), bf16)
    for i in range(NB):
        z_s[1, i] = jnp.zeros((NF, 128), bf16)

    for c in small:
        c.wait()
    eye = (lax.broadcasted_iota(jnp.int32, (8, KS), 0)
           == lax.broadcasted_iota(jnp.int32, (8, KS), 1)).astype(bf16)
    taps = lax.dot_general(eye, shift_s[...], (((1,), (1,)), ((), ())),
                           preferred_element_type=f32)
    row8 = lax.broadcasted_iota(jnp.int32, (8, D), 0)
    dv = jnp.broadcast_to(dvec_s[...].astype(f32), (8, D))
    prm = jnp.where(row8 == KS, dv, taps)
    gw = gate_s[...].astype(f32)
    for n in range(NC):
        prm_s[n] = prm[:, n * 128:(n + 1) * 128]
        gw_s[n] = jnp.broadcast_to(gw[:, n * 128:(n + 1) * 128], (8, 128))

    def relayout_t(slot):
        for p in range(8):
            blk = stage[slot, p * 128:(p + 1) * 128]
            tmpu[p * 512:(p + 1) * 512, :] = pltpu.bitcast(
                blk.reshape(128 * HC, 128), u32)

    def relayout_r(chunk, j):
        for p in range(8):
            e = tmpu[pl.ds(p * 512 + j, 64, stride=8), :]
            o = tmpu[pl.ds(p * 512 + 4 + j, 64, stride=8), :]
            w_s[chunk * HC + 2 * j, p * 64:(p + 1) * 64, :] = (
                (e & jnp.uint32(0xFFFF)) | (o << 16))
            w_s[chunk * HC + 2 * j + 1, p * 64:(p + 1) * 64, :] = (
                (e >> 16) | (o & jnp.uint32(0xFFFF0000)))

    def wtile(n):
        return pltpu.bitcast(w_s[n], bf16)

    w_copy(0, 0, 0).wait()
    relayout_t(0)
    for j in range(HC // 2):
        relayout_r(0, j)
    for n in range(NC):
        x0_copy(n).wait()

    def pre_body(i, carry):
        nxt = jnp.minimum(i + 1, NCH - 1)
        nslot = nxt % 3

        @pl.when(i + 1 < NCH)
        def _():
            w_copy(0, 0, nslot).wait()

        for m in range(3):
            @pl.when(jnp.logical_and(i + 3 < NCH, (i + 3) // 4 == m))
            def _(m=m):
                w_copy(m, (i + 3) % 4, i % 3).start()

        for gi, group in enumerate(pre_groups):
            @pl.when(i == gi)
            def _(group=group):
                for c in group:
                    c.start()

        sc = jnp.where(i < NCH // 3, scale, 1.0).astype(f32)
        relayout_t(nslot)
        for j in range(HC // 2):
            for hh in range(2):
                n = i * HC + 2 * j + hh
                xb = jnp.concatenate([x_s[t, 0:BULK, :] for t in range(NC)], axis=1)
                r = jnp.dot(xb, wtile(n), preferred_element_type=f32) * sc
                qkv_s[n, 0:BULK, :] = r.astype(bf16)
            relayout_r(nxt, j)
        return carry

    lax.fori_loop(0, NCH, pre_body, 0)

    for group in pre_groups:
        for c in group:
            c.wait()
    for c in late:
        c.start()

    def conv_filter_dft(ct, r, slot):
        c0 = pl.multiple_of(ct * 128, 128)
        for jj in range(2):
            d = 2 * r + jj
            kf_s[slot, d] = lax.dot_general(
                fw_s[...], f_s[d, pl.ds(c0, 128), :], (((1,), (1,)), ((), ())),
                preferred_element_type=f32)

    def conv_kv(ct, r):
        r0 = pl.multiple_of(r * 2 * BL, 2 * BL)
        prm = prm_s[ct]
        kk = k_s[ct, pl.ds(r0, 2 * BL + PAD), :].astype(f32)
        ks = kk[PAD:] * prm[0:1]
        for tau in range(1, KS):
            ks = ks + kk[PAD - tau:2 * BL + PAD - tau] * prm[tau:tau + 1]
        kv = (ks * v_s[ct, pl.ds(r0, 2 * BL), :].astype(f32)).astype(bf16)
        kv_s[ct, pl.ds(r0, 2 * BL), :] = kv
        return kv

    def conv_kv_dft(kv, r, slot):
        for jj in range(2):
            u_s[slot, 2 * r + jj] = jnp.dot(
                fw_s[...], kv[jj * BL:(jj + 1) * BL], preferred_element_type=f32)

    def conv_products(r, slot):
        for par in range(2):
            ore = pl.multiple_of(r * 32 + 8 * par, 8)
            oim = pl.multiple_of(r * 32 + 16 + 8 * par, 8)
            prev = None
            for bi in range(4):
                acc = [None] * 4
                for bj in range(bi + 1):
                    us = [(u_s[slot, 4 * bj + t, pl.ds(ore, 8), :],
                           u_s[slot, 4 * bj + t, pl.ds(oim, 8), :]) for t in range(4)]
                    d0 = 4 * (bi - bj)
                    ks = {d: (kf_s[slot, d, pl.ds(ore, 8), :],
                              kf_s[slot, d, pl.ds(oim, 8), :])
                          for d in range(max(d0 - 3, 0), d0 + 4)}
                    for ti in range(4):
                        for tj in range(4):
                            d = d0 + ti - tj
                            if d < 0:
                                continue
                            kr, ki = ks[d]
                            ur, ui = us[tj]
                            pr = kr * ur - ki * ui
                            pi = kr * ui + ki * ur
                            if acc[ti] is None:
                                acc[ti] = (pr, pi)
                            else:
                                acc[ti] = (acc[ti][0] + pr, acc[ti][1] + pi)
                for ti in range(4):
                    yr, yi = acc[ti]
                    if prev is None:
                        zr, zi = yr, yi
                    elif par == 0:
                        zr, zi = yr - prev[1], yi + prev[0]
                    else:
                        zr, zi = yr + prev[1], yi - prev[0]
                    prev = (yr, yi)
                    z_s[slot, 4 * bi + ti, pl.ds(ore, 8), :] = zr.astype(bf16)
                    z_s[slot, 4 * bi + ti, pl.ds(oim, 8), :] = zi.astype(bf16)

    def conv_inverse(ct, r, slot):
        dvec = prm_s[ct][KS:KS + 1]
        for jj in range(2):
            i = 2 * r + jj
            r0 = pl.multiple_of(i * BL, BL)
            y = jnp.dot(fi_s[...], z_s[slot, i], preferred_element_type=f32)
            y = y + kv_s[ct, pl.ds(r0, BL), :].astype(f32) * dvec
            a = x_s[ct, pl.ds(r0, BL), :].astype(f32) * y
            a_s[ct, pl.ds(r0, BL), :] = a.astype(bf16)

    def conv_prologue(r, carry):
        conv_filter_dft(0, r, 0)
        conv_kv_dft(conv_kv(0, r), r, 0)
        return carry

    lax.fori_loop(0, 8, conv_prologue, 0)

    wo_u = wo_s.bitcast(u32)

    def step(s, carry):
        @pl.when(s == 8)
        def _():
            for c in late:
                c.wait()

        row = lax.broadcasted_iota(jnp.int32, (LTOT, LTOT), 0)
        col = lax.broadcasted_iota(jnp.int32, (LTOT, LTOT), 1)
        mask = (row >= SEG) | (col >= SEG) | (col <= row)

        ct = s >> 3
        r = s & 7
        cnext = jnp.minimum(ct + 1, NC - 1)
        cprev = jnp.maximum(ct - 1, 0)
        slot = ct & 1
        oslot = 1 - slot

        t0 = pl.multiple_of(BULK + TP * s, 8)
        wpos = [pl.multiple_of(_ring(BULK + TP * s + 8 * j), 8) for j in range(TP // 8)]
        rpos = pl.multiple_of(_ring(SEG * s), SEG)
        lpos = pl.multiple_of(_ring(TP * s), 8)
        bpos = pl.multiple_of(TP * s, 8)
        gpos = pl.multiple_of(SEG * s, SEG)

        lhs = jnp.concatenate(
            [jnp.concatenate([x_s[t, pl.ds(t0, TP), :] for t in range(NC)], axis=1),
             mem_s[...]], axis=0)

        memq = [None] * H
        omem = [None] * H
        pend = [None] * H
        ld = [None] * H
        pv_in = [None] * H
        acc = [None] * NC
        l2s = {}

        def qkv_mm(h):
            rq = (jnp.dot(lhs, wtile(h), preferred_element_type=f32) * scale).astype(bf16)
            rk = jnp.dot(lhs, wtile(H + h), preferred_element_type=f32).astype(bf16)
            rv = jnp.dot(lhs, wtile(2 * H + h), preferred_element_type=f32).astype(bf16)
            pend[h] = (rq, rk, rv)
            memq[h] = (rq[TP:], rk[TP:], rv[TP:])

        def qkv_st(h):
            for m in range(3):
                for j in range(TP // 8):
                    qkv_s[m * H + h, pl.ds(wpos[j], 8), :] = pend[h][m][8 * j:8 * j + 8]

        def att_ld(h):
            ld[h] = [qkv_s[m * H + h, pl.ds(rpos, SEG), :] for m in range(3)]

        def att_qk(h):
            q, k, v = [jnp.concatenate([ld[h][m], memq[h][m]], axis=0) for m in range(3)]
            sc = lax.dot_general(q, k, (((1,), (1,)), ((), ())),
                                 preferred_element_type=f32)
            sc = jnp.where(mask, sc, -1e9)
            mx = jnp.max(sc, axis=-1, keepdims=True)
            p = jnp.exp(sc - mx)
            den = jnp.sum(p, axis=-1, keepdims=True)
            pv_in[h] = (p.astype(bf16), v, 1.0 / den)

        def att_pv(h):
            p, v, rl = pv_in[h]
            o = (jnp.dot(p, v, preferred_element_type=f32) * rl).astype(bf16)
            o_s[h, pl.ds(rpos, SEG), :] = o[:SEG]
            omem[h] = o[SEG:]

        def wo_ld(g):
            l2s[g] = [o_s[h, pl.ds(lpos, TP), :] for h in range(g * G, (g + 1) * G)]

        def wo_mm(g):
            h0 = g * G
            l2 = jnp.concatenate(
                [jnp.concatenate([l2s[g][h - h0], omem[h]], axis=0)
                 for h in range(h0, h0 + G)], axis=1)
            for n in range(NC):
                w = pltpu.bitcast(wo_u[n, h0 * DH // 2:(h0 + G) * DH // 2, :], bf16)
                res = jnp.dot(l2, w, preferred_element_type=f32)
                acc[n] = res if acc[n] is None else acc[n] + res

        def gate():
            tot = None
            for n in range(NC):
                xv = x_s[n, pl.ds(gpos, SEG), :].astype(f32) * gw_s[n][0:1]
                tot = xv if tot is None else tot + xv
            z = jnp.sum(tot, axis=-1, keepdims=True)
            g_s[pl.ds(gpos, SEG), :] = jnp.broadcast_to(jax.nn.sigmoid(z), (SEG, 128))

        def grp(g):
            return range(g * G, (g + 1) * G)

        conv_inverse(cprev, r, oslot)
        conv_filter_dft(cnext, r, oslot)
        kv_new = conv_kv(cnext, r)
        gate()
        for g in range(NG + 3):
            if 0 <= g - 1 < NG:
                for h in grp(g - 1):
                    att_ld(h)
            if 0 <= g - 3 < NG:
                wo_ld(g - 3)
            if g < NG:
                for h in grp(g):
                    qkv_mm(h)
                for h in grp(g):
                    qkv_st(h)
            if g == 0:
                conv_kv_dft(kv_new, r, oslot)
                conv_products(r, slot)
            if 0 <= g - 1 < NG:
                for h in grp(g - 1):
                    att_qk(h)
            if 0 <= g - 2 < NG:
                for h in grp(g - 2):
                    att_pv(h)
            if 0 <= g - 3 < NG:
                wo_mm(g - 3)
        for n in range(NC):
            res = acc[n].astype(bf16)
            b_s[n, pl.ds(bpos, TP), :] = res[:TP]
            mem_s[:, n * 128:(n + 1) * 128] = res[TP:]
        return carry

    lax.fori_loop(0, NSEG, step, 0)

    P0 = TP * NSEG
    q0 = P0 % RING
    n1 = RING - q0

    def post_body(n, carry):
        conv_inverse(NC - 1, n, (NC - 1) & 1)
        l2 = jnp.concatenate(
            [jnp.concatenate([o_s[h, q0:RING, :], o_s[h, 0:BULK - n1, :]], axis=0)
             for h in range(H)], axis=1)
        tail = jnp.dot(l2, pltpu.bitcast(wo_u[n], bf16), preferred_element_type=f32)
        tail = tail.astype(bf16).astype(f32)
        for p in range(S // 256):
            rows = slice(p * 256, (p + 1) * 256)
            g = g_s[rows, :]
            a = a_s[n, rows, :].astype(f32)
            if p * 256 < P0:
                b = b_s[n, rows, :].astype(f32)
            else:
                b = tail[p * 256 - P0:(p + 1) * 256 - P0]
            b_s[n, rows, :] = (g * a + (1.0 - g) * b).astype(bf16)
        out_copy(n).start()
        return carry

    lax.fori_loop(0, NC, post_body, 0)
    for n in range(NC):
        out_copy(n).wait()


@functools.partial(jax.jit, static_argnames=("B_seg_len",))
def pallas_gated_mix__ssm_conv_h3__memory_aug_recurrent_mem_tr__prompt_kernel(
    A_q: jax.Array,
    A_k: jax.Array,
    A_v: jax.Array,
    A_shift_k: jax.Array,
    A_ssm_k: jax.Array,
    A_ssm_D: jax.Array,
    B_x: jax.Array,
    B_mem0: jax.Array,
    B_Wq: jax.Array,
    B_Wk: jax.Array,
    B_Wv: jax.Array,
    B_Wo: jax.Array,
    B_seg_len,
    gate_w: jax.Array,
):
    del B_x
    assert int(B_seg_len) == SEG
    assert A_q.shape == (1, S, D) and B_Wq.shape == (D, H, DH)
    assert B_mem0.shape == (1, M, D) and A_shift_k.shape == (D, KS)

    n_pre = NB + 4 + NC + NC
    scratch = [
        pltpu.VMEM((NC, S, 128), bf16),
        pltpu.VMEM((NC, S + PAD, 128), bf16),
        pltpu.VMEM((NC, S, 128), bf16),
        pltpu.VMEM((NB, D, 128), bf16),
        pltpu.VMEM((NC, S, 128), bf16),
        pltpu.VMEM((NC, S, 128), bf16),
        pltpu.VMEM((NC, S, 128), bf16),
        pltpu.VMEM((S, 128), f32),
        pltpu.VMEM((3 * H, D // 2, 128), u32),
        pltpu.VMEM((NC, H * DH, 128), bf16),
        pltpu.VMEM((3, D, HC, 128), bf16),
        pltpu.VMEM((D * HC // 2, 128), u32),
        pltpu.VMEM((3 * H, RING, 128), bf16),
        pltpu.VMEM((H, RING, 128), bf16),
        pltpu.VMEM((2, NB, NF, 128), f32),
        pltpu.VMEM((2, NB, NF, 128), f32),
        pltpu.VMEM((2, NB, NF, 128), bf16),
        pltpu.VMEM((NF, BL), bf16),
        pltpu.VMEM((BL, NF), bf16),
        pltpu.VMEM((M, D), bf16),
        pltpu.VMEM((D, KS), bf16),
        pltpu.VMEM((1, D), bf16),
        pltpu.VMEM((1, D), bf16),
        pltpu.VMEM((NC, 8, 128), f32),
        pltpu.VMEM((NC, 8, 128), f32),
        pltpu.SemaphoreType.DMA((3,)),
        pltpu.SemaphoreType.DMA((NC,)),
        pltpu.SemaphoreType.DMA((4,)),
        pltpu.SemaphoreType.DMA((n_pre,)),
        pltpu.SemaphoreType.DMA((2 * (NC - 2),)),
        pltpu.SemaphoreType.DMA((NC,)),
    ]
    out = pl.pallas_call(
        _kernel,
        out_shape=jax.ShapeDtypeStruct((S, D), bf16),
        in_specs=[pl.BlockSpec(memory_space=pl.ANY)] * 12,
        out_specs=pl.BlockSpec(memory_space=pl.ANY),
        scratch_shapes=scratch,
        compiler_params=pltpu.CompilerParams(vmem_limit_bytes=124 * 1024 * 1024),
    )(
        A_q.reshape(S, D), A_k.reshape(S, D), A_v.reshape(S, D),
        A_shift_k, A_ssm_k, A_ssm_D.reshape(1, D), B_mem0.reshape(M, D),
        B_Wq, B_Wk, B_Wv, B_Wo.reshape(H * DH, D), gate_w.reshape(1, D),
    )
    return out.reshape(1, S, D)
```

```python
import functools
import math
import os

import jax
import jax.numpy as jnp
from jax import lax
import jax.experimental.pallas as pl
import jax.experimental.pallas.tpu as pltpu

bf16 = jnp.bfloat16
f32 = jnp.float32
u32 = jnp.uint32

S = 2048
D = 1024
H = 32
DH = 128
M = 8
SEG = 32
NSEG = S // SEG
KS = 4
TP = 24
BULK = S - TP * NSEG
P0 = TP * NSEG
RING = 576
NC = D // 128
BL = 128
NB = S // BL
NF = 2 * BL
G = 8
HC = 8
NCH = 3 * H // HC
PAD = 16
LTOT = SEG + M
NSLOT = 4
RP = 16
KVP = 32
UNROLL = int(os.environ.get("UNROLL", 2))
UA = int(os.environ.get("UA", 0))
UC = int(os.environ.get("UC", 1))
POSTU = int(os.environ.get("POSTU", 1))


def _make_plan():
    nq, kper, koff = [int(t) for t in os.environ.get("PLANV", "72,12,3").split(",")]
    plan = {}
    done = 0
    for i in range(nq):
        tgt = (i + 1) * 144 // nq
        plan[i] = (tgt - done, 0)
        done = tgt
    for j in range(2 * BL // KVP):
        i = koff + j * kper
        plan[i] = (plan.get(i, (0, 0))[0], 1)
    return plan


PLAN = _make_plan()


def _ring(x):
    x = jnp.where(x >= 2 * RING, x - 2 * RING, x)
    return jnp.where(x >= RING, x - RING, x)


def _kernel(x_hbm, k_hbm, v_hbm, shift_hbm, filt_hbm, dvec_hbm, mem0_hbm,
            wq_hbm, wk_hbm, wv_hbm, wo_hbm, gate_hbm,
            out_hbm,
            x_s, kin_s, f_s, kv_s, abg_s,
            w0_s, w1_s, wo_s, stage, tmpu, qkv0_s, qkv1_s, o0_s, o1_s,
            uk_s, z_s, fw_s, fi_s, p_s, acc_s,
            mem_s, shift_s, dvec_s, gate_s, prm_s, zero_s,
            sem_w, sem_x0, sem_pre, sem_late, sem_out):
    scale = DH ** (-0.5)
    w_hbms = (wq_hbm, wk_hbm, wv_hbm)
    w_bufs = (w0_s, w1_s)
    qkv_rings = (qkv0_s, qkv1_s)
    o_rings = (o0_s, o1_s)

    def ring_of(h):
        g = h // G
        return g % 2, (g // 2) * G + h % G

    sem_idx = [0]

    def next_sem():
        sem_idx[0] += 1
        return sem_pre.at[sem_idx[0] - 1]

    def x0_copy(n):
        return pltpu.make_async_copy(
            x_hbm.at[pl.ds(0, BULK), pl.ds(n * 128, 128)],
            x_s.at[n, pl.ds(0, BULK), :], sem_x0.at[n])

    def w_copy(c, slot):
        return pltpu.make_async_copy(
            w_hbms[c // 4].at[:, pl.ds((c % 4) * HC, HC), :],
            stage.at[slot, pl.ds(0, D)], sem_w.at[slot])

    def kv_copies(n, sem_k, sem_v):
        return [
            pltpu.make_async_copy(k_hbm.at[:, pl.ds(n * 128, 128)],
                                  kin_s.at[0, n, pl.ds(PAD, S), :], sem_k),
            pltpu.make_async_copy(v_hbm.at[:, pl.ds(n * 128, 128)],
                                  kin_s.at[1, n, pl.ds(PAD, S), :], sem_v),
        ]

    def filt_copy(d):
        return pltpu.make_async_copy(filt_hbm.at[:, pl.ds(d * 128, 128)],
                                     f_s.at[d], next_sem())

    def xrest_copy(n):
        return pltpu.make_async_copy(
            x_hbm.at[pl.ds(BULK, S - BULK), pl.ds(n * 128, 128)],
            x_s.at[n, pl.ds(BULK, S - BULK), :], next_sem())

    def wo_copy(n):
        return pltpu.make_async_copy(wo_hbm.at[:, pl.ds(n * 128, 128)],
                                     wo_s.at[n], next_sem())

    conv_groups = [
        [filt_copy(d) for d in range(0, NB // 2)],
        [filt_copy(d) for d in range(NB // 2, NB)],
        kv_copies(0, next_sem(), next_sem()) + [
            pltpu.make_async_copy(mem0_hbm, mem_s, next_sem()),
            pltpu.make_async_copy(shift_hbm, shift_s, next_sem()),
            pltpu.make_async_copy(dvec_hbm, dvec_s, next_sem()),
            pltpu.make_async_copy(gate_hbm, gate_s, next_sem()),
        ],
    ]
    main_groups = [
        kv_copies(1, next_sem(), next_sem()) + [xrest_copy(n) for n in range(0, 3)],
        [xrest_copy(n) for n in range(3, NC)],
    ] + [[wo_copy(2 * q), wo_copy(2 * q + 1)] for q in range(4)]
    pre_groups = conv_groups + main_groups
    late = []
    for n in range(2, NC):
        late += kv_copies(n, sem_late.at[0], sem_late.at[0])
    late_dst = kin_s.at[:, pl.ds(2, NC - 2), pl.ds(PAD, S), :]
    late_all = pltpu.make_async_copy(late_dst, late_dst, sem_late.at[0])

    def out_copy(n, tail):
        rows = pl.ds(P0, S - P0) if tail else pl.ds(0, P0)
        return pltpu.make_async_copy(abg_s.at[NC + n, rows, :],
                                     out_hbm.at[rows, pl.ds(n * 128, 128)],
                                     sem_out.at[2 * n + tail])

    def dft_table(shape, rho_axis, row0):
        row = lax.broadcasted_iota(jnp.int32, shape, 0) + row0
        col = lax.broadcasted_iota(jnp.int32, shape, 1)
        rho, t = (row, col) if rho_axis == 0 else (col, row)
        f = ((rho >> 5) << 4) + ((rho & 7) << 1) + ((rho >> 3) & 1)
        im = (rho >> 4) & 1
        ph = ((2 * f + 1) * t + im * BL) & (4 * BL - 1)
        ph = jnp.where(ph > 2 * BL, 4 * BL - ph, ph)
        return jnp.cos(ph.astype(f32) * (math.pi / NF))

    def fw_body(i, carry):
        r0 = pl.multiple_of(i * BL, BL)
        fw_s[pl.ds(r0, BL), :] = dft_table((BL, BL), 0, r0).astype(bf16)
        return carry

    def fi_body(i, carry):
        r0 = pl.multiple_of(i * (BL // 2), BL // 2)
        fi_s[pl.ds(r0, BL // 2), :] = (
            dft_table((BL // 2, NF), 1, r0) * (1.0 / BL)).astype(bf16)
        return carry

    w_copy(0, 0).start()
    zero_s[0] = 0
    lax.fori_loop(0, 2, fw_body, 0)
    for n in range(NC):
        x0_copy(n).start()
    lax.fori_loop(0, 2, fi_body, 0)
    w_copy(1, 1).start()
    for n in range(NC):
        kin_s[0, n, 0:PAD, :] = jnp.zeros((PAD, 128), bf16)
    if not UA:
        for i in range(NB):
            z_s[1, i] = jnp.zeros((NF, 128), bf16)
    zero = zero_s[0]

    def conv_filter_dft(ct, d, slot):
        c0 = ct * 128 if isinstance(ct, int) else pl.multiple_of(ct * 128, 128)
        uk_s[(2 * slot + 1) * NB + d] = lax.dot_general(
            fw_s[...], f_s[d, pl.ds(c0, 128), :], (((1,), (1,)), ((), ())),
            preferred_element_type=f32)

    def conv_kv(ct, row0):
        kk = kin_s[0, ct, pl.ds(row0, KVP + PAD), :].astype(f32)
        ks = kk[PAD:] * prm_s[ct, 0, 0:1, :]
        for tau in range(1, KS):
            ks = ks + kk[PAD - tau:KVP + PAD - tau] * prm_s[ct, tau, 0:1, :]
        vv = kin_s[1, ct, pl.ds(row0 + PAD, KVP), :].astype(f32)
        kv_s[ct, pl.ds(row0, KVP), :] = (ks * vv).astype(bf16)

    def kv_anchor(pos, val):
        kin_s[0, 0, pl.ds(S + PAD + pos, 8), :] = val

    def conv_kv_dft(ct, j, slot):
        r0 = j * BL if isinstance(j, int) else pl.multiple_of(j * BL, BL)
        uk_s[2 * slot * NB + j] = jnp.dot(
            fw_s[...], kv_s[ct, pl.ds(r0, BL), :], preferred_element_type=f32)

    def conv_products(r, slot):
        ub = 2 * slot * NB
        kb = ub + NB

        def cmac(acc, k, u):
            pr = k[0] * u[0] - k[1] * u[1]
            pi = k[0] * u[1] + k[1] * u[0]
            return (pr, pi) if acc is None else (acc[0] + pr, acc[1] + pi)

        for par in range(2):
            ore = pl.multiple_of(r * 32, 32) + 8 * par
            oim = pl.multiple_of(r * 32, 32) + (16 + 8 * par)

            def load(idx):
                return (uk_s[idx, pl.ds(ore, 8), :], uk_s[idx, pl.ds(oim, 8), :])

            prev = None
            for i in range(0, NB, 2):
                y0 = y1 = None
                khi = load(kb + i + 1)
                for j in range(i + 2):
                    u = load(ub + j)
                    y1 = cmac(y1, khi, u)
                    if j <= i:
                        khi = load(kb + i - j)
                        y0 = cmac(y0, khi, u)
                    if j < i + 1:
                        yield
                for ii, y in ((i, y0), (i + 1, y1)):
                    if prev is None:
                        zr, zi = y
                    elif par == 0:
                        zr, zi = y[0] - prev[1], y[1] + prev[0]
                    else:
                        zr, zi = y[0] + prev[1], y[1] - prev[0]
                    prev = y
                    z_s[slot, ii, pl.ds(ore, 8), :] = zr.astype(bf16)
                    z_s[slot, ii, pl.ds(oim, 8), :] = zi.astype(bf16)
                yield

    def conv_inverse(ct, r, slot):
        dvec = prm_s[ct, KS, 0:1, :]
        for jj in range(2):
            i = 2 * r + jj
            r0 = pl.multiple_of(i * BL, BL)
            y = jnp.dot(fi_s[...], z_s[slot, i], preferred_element_type=f32)
            y = y + kv_s[ct, pl.ds(r0, BL), :].astype(f32) * dvec
            a = x_s[ct, pl.ds(r0, BL), :].astype(f32) * y
            abg_s[ct, pl.ds(r0, BL), :] = a.astype(bf16)

    NPIECE = D // RP

    def relayout(par, half, slot, p):
        t0 = (p % 8) * (RP * HC // 2)
        blk = stage[slot, p * RP:(p + 1) * RP]
        tmpu[t0:t0 + RP * HC // 2, :] = pltpu.bitcast(blk.reshape(RP * HC, 128), u32)
        for j in range(HC // 2):
            e = tmpu[pl.ds(t0 + j, RP // 2, stride=8), :]
            o = tmpu[pl.ds(t0 + 4 + j, RP // 2, stride=8), :]
            rows = slice(p * RP // 2, (p + 1) * RP // 2)
            w_bufs[par][half * HC + 2 * j, rows, :] = (
                (e & jnp.uint32(0xFFFF)) | (o << 16))
            w_bufs[par][half * HC + 2 * j + 1, rows, :] = (
                (e >> 16) | (o & jnp.uint32(0xFFFF0000)))

    def wtile(n):
        c = n // HC
        return pltpu.bitcast(w_bufs[c % 2][(c // 2) * HC + n % HC], bf16)

    x_u = x_s.bitcast(u32)

    def bulk_dot(par, half, hh):
        xb = jnp.concatenate(
            [pltpu.bitcast(x_u[t, 0:BULK // 2, :], bf16) for t in range(NC)], axis=1)
        w = pltpu.bitcast(w_bufs[par][half * HC + hh], bf16)
        r = jnp.dot(xb, w, preferred_element_type=f32).astype(bf16)
        qkv_rings[par][(half // 2) * (H // 2) + (half % 2) * G + hh, 0:BULK, :] = r
        return r

    def start_copies(cond):
        def start(pred, make):
            def go():
                for c in make():
                    c.start()
            if pred is True:
                go()
            elif pred is not False:
                pl.when(pred)(go)

        for c in range(NCH - NSLOT):
            start(cond(c), lambda: [w_copy(c + NSLOT, c % NSLOT)])
        for gi, group in enumerate(pre_groups):
            start(cond(gi + 2), lambda: group)

    def chunk_dots(par, half, aslot, nhalf, nslot, first):
        for hh in range(HC):
            if hh == first and first > 0:
                w_copy(0, nslot).wait()
            r = bulk_dot(par, half, hh)
            if hh >= first:
                p0 = (hh - first) * NPIECE // (HC - first)
                p1 = (hh - first + 1) * NPIECE // (HC - first)
                for p in range(p0, p1):
                    q0 = ((p - p0) * (BULK // HC) // (p1 - p0)) * HC
                    stage[aslot, D] = r[q0:q0 + HC]
                    relayout(1 - par, nhalf, nslot, p)

    w_copy(0, 0).wait()
    w_copy(2, 2).start()
    for p in range(NPIECE):
        relayout(0, 0, 0, p)
    for n in range(NC):
        x0_copy(n).wait()
        if n == 0:
            w_copy(3, 3).start()
    start_copies(lambda c: c == 0)
    chunk_dots(0, 0, zero, 0, 1, int(os.environ.get('FIRST', 4)))

    def pre_body(k, carry):
        for par in (1, 0):
            i = 2 * k + 2 - par
            nslot = (i + 1) % NSLOT
            w_copy(0, nslot).wait()
            start_copies(lambda c: (i == c) if (c % 2 == par and c > 0) else False)
            chunk_dots(par, k + 1 - par, i % NSLOT, k + 1, nslot, 0)
        return carry

    lax.fori_loop(0, NCH // 2 - 1, pre_body, 0)

    for group in conv_groups:
        for c in group:
            c.wait()
    for c in late:
        c.start()
    taps = shift_s[...].astype(f32)
    dv = dvec_s[...].astype(f32)
    gw = gate_s[...].astype(f32)
    for n in range(NC):
        for tau in range(KS):
            prm_s[n, tau] = jnp.broadcast_to(
                taps[tau:tau + 1, n * 128:(n + 1) * 128], (8, 128))
        prm_s[n, KS] = jnp.broadcast_to(dv[n:n + 1], (8, 128))
        prm_s[n, KS + 1] = jnp.broadcast_to(gw[n:n + 1], (8, 128))

    zpos = pl.multiple_of(zero * 8, 8)
    for hh in range(HC):
        r = bulk_dot(1, NCH // 2 - 1, hh)
        for q in range(2 * BL // KVP):
            kv_anchor(zpos, r[q * KVP * 2:q * KVP * 2 + 8])
            conv_kv(0, 2 * BL * hh + KVP * q)
        for d in (2 * hh, 2 * hh + 1):
            conv_filter_dft(0, d, 0)
        if hh > 0:
            for j in (2 * hh - 2, 2 * hh - 1):
                conv_kv_dft(0, j, 0)
    for j in (NB - 2, NB - 1):
        conv_kv_dft(0, j, 0)
    for group in main_groups:
        for c in group:
            c.wait()

    wo_u = wo_s.bitcast(u32)

    def step(s, mem, do_inv, do_fwd):
        row = lax.broadcasted_iota(jnp.int32, (2 * LTOT, 2 * LTOT), 0)
        col = lax.broadcasted_iota(jnp.int32, (2 * LTOT, 2 * LTOT), 1)
        row_mem = row >= 2 * SEG
        col_mem = col >= 2 * SEG
        row_head = jnp.where(row_mem, (row - 2 * SEG) // M, row // SEG)
        col_head = jnp.where(col_mem, (col - 2 * SEG) // M, col // SEG)
        same = row_head == col_head
        mask = same & (row_mem | col_mem | (col <= row))
        fill = jnp.where(same, -1e9 / scale, -jnp.inf).astype(f32)

        ct = s >> 3
        r = s & 7
        cnext = jnp.minimum(ct + 1, NC - 1)
        cprev = jnp.maximum(ct - 1, 0)
        slot = ct & 1
        oslot = 1 - slot

        t0 = pl.multiple_of(BULK + TP * s, 8)
        wpos = [pl.multiple_of(_ring(BULK + TP * s + 8 * j), 8) for j in range(TP // 8)]
        rpos = pl.multiple_of(_ring(SEG * s), SEG)
        lpos = pl.multiple_of(_ring(TP * s), 8)
        bpos = pl.multiple_of(TP * s, 8)
        gpos = pl.multiple_of(SEG * s, SEG)
        apos = pl.multiple_of(r * 8, 8)
        kpos = pl.multiple_of((r & 1) * 8, 8)

        lhs = jnp.concatenate(
            [jnp.concatenate([x_s[t, pl.ds(t0, TP), :] for t in range(NC)], axis=1),
             mem], axis=0)

        memq = [None] * H
        omem = [None] * H
        pv_in = [None] * H
        acc = [None] * NC

        prods = conv_products(r, slot)
        kv_rows = [pl.multiple_of(r * 2 * BL + q * KVP, KVP)
                   for q in range(2 * BL // KVP)] if do_fwd else []

        def release(key, res):
            n_prod, n_kv = PLAN.get(key, (0, 0))
            if n_prod:
                uk_s[4 * NB, pl.ds(apos, 8), :] = res[0:8]
                for _ in range(n_prod):
                    next(prods, None)
            if n_kv and kv_rows:
                kv_anchor(kpos, res[0:8].astype(bf16))
                conv_kv(cnext, kv_rows.pop(0))

        def qkv(h):
            ri, t = ring_of(h)
            memq[h] = []
            for m in range(3):
                res = jnp.dot(lhs, wtile(m * H + h), preferred_element_type=f32)
                release(3 * h + m, res)
                res = res.astype(bf16)
                for j in range(TP // 8):
                    qkv_rings[ri][m * (H // 2) + t, pl.ds(wpos[j], 8), :] = (
                        res[8 * j:8 * j + 8])
                memq[h].append(res[TP:])

        def att_qk(h):
            ri, t = ring_of(h)
            q, k, v = [
                jnp.concatenate(
                    [qkv_rings[ri][m * (H // 2) + t, pl.ds(rpos, SEG), :],
                     qkv_rings[ri][m * (H // 2) + t + 1, pl.ds(rpos, SEG), :],
                     memq[h][m], memq[h + 1][m]], axis=0) for m in range(3)]
            sc = lax.dot_general(q, k, (((1,), (1,)), ((), ())),
                                 preferred_element_type=f32)
            sc = jnp.where(mask, sc, fill)
            mx = jnp.max(sc, axis=-1, keepdims=True)
            p = jnp.exp2((sc - mx) * (scale * math.log2(math.e)))
            den = jnp.sum(p, axis=-1, keepdims=True)
            rl = pl.reciprocal(den, approx=True)
            rl = rl * (2.0 - den * rl)
            p_s[h // 2] = p.astype(bf16)
            pv_in[h] = (v, rl)

        def att_pv(h):
            ri, t = ring_of(h)
            v, rl = pv_in[h]
            o = (jnp.dot(p_s[h // 2], v, preferred_element_type=f32) * rl).astype(bf16)
            o_rings[ri][t, pl.ds(rpos, SEG), :] = o[:SEG]
            o_rings[ri][t + 1, pl.ds(rpos, SEG), :] = o[SEG:2 * SEG]
            omem[h] = o[2 * SEG:2 * SEG + M]
            omem[h + 1] = o[2 * SEG + M:]

        def wo_grp(g):
            h0 = g * G
            parts = []
            for h in range(h0, h0 + G):
                ri, t = ring_of(h)
                parts.append(jnp.concatenate(
                    [o_rings[ri][t, pl.ds(lpos, TP), :], omem[h]], axis=0))
            l2 = jnp.concatenate(parts, axis=1)
            for n in range(NC):
                w = pltpu.bitcast(wo_u[n, h0 * DH // 2:(h0 + G) * DH // 2, :], bf16)
                res = jnp.dot(l2, w, preferred_element_type=f32)
                if g == 0:
                    acc_s[n] = res
                else:
                    acc[n] = (acc_s[n] if g == 1 else acc[n]) + res

        def gate():
            tot = None
            for n in range(NC):
                xv = x_s[n, pl.ds(gpos, SEG), :].astype(f32) * prm_s[n, KS + 1, 0:1, :]
                tot = xv if tot is None else tot + xv
            z = jnp.sum(tot, axis=-1, keepdims=True)
            abg_s[2 * NC, pl.ds(gpos, SEG), :] = jnp.broadcast_to(
                jax.nn.sigmoid(z), (SEG, 128)).astype(bf16)

        def qkv_grp(g):
            for h in range(g * G, (g + 1) * G):
                qkv(h)

        def qk_grp(g):
            for h in range(g * G, (g + 1) * G, 2):
                att_qk(h)

        def pv_grp(g):
            for h in range(g * G, (g + 1) * G, 2):
                att_pv(h)

        if do_inv:
            conv_inverse(cprev, r, oslot)
        qkv_grp(0)
        qkv_grp(1)
        qk_grp(0)
        qkv_grp(2)
        pv_grp(0)
        qk_grp(1)
        qkv_grp(3)
        gate()
        pv_grp(1)
        qk_grp(2)
        wo_grp(0)
        pv_grp(2)
        qk_grp(3)
        wo_grp(1)
        pv_grp(3)
        wo_grp(2)
        wo_grp(3)
        for _ in prods:
            pass
        assert not kv_rows
        if do_fwd:
            for jj in range(2):
                conv_filter_dft(cnext, 2 * r + jj, oslot)
            for jj in range(2):
                conv_kv_dft(cnext, 2 * r + jj, oslot)
        new_mem = []
        for n in range(NC):
            res = acc[n].astype(bf16)
            abg_s[NC + n, pl.ds(bpos, TP), :] = res[:TP]
            new_mem.append(res[TP:])
        return jnp.concatenate(new_mem, axis=1)

    def steps(it, carry, unroll, do_inv=True, do_fwd=True, wait_late=False):
        if wait_late:
            @pl.when(it == 8 // unroll)
            def _():
                late_all.wait()

        mem = mem_s[...]
        for u in range(unroll):
            mem = step(it * unroll + u, mem, do_inv, do_fwd)
        mem_s[...] = mem
        return carry

    lo, hi = 0, NSEG
    if UA:
        steps_a = functools.partial(steps, unroll=UA, do_inv=False)
        lax.fori_loop(0, 8 // UA, steps_a, 0)
        late_all.wait()
        lo = 8
    if UC:
        hi = NSEG - 8
    steps_b = functools.partial(steps, unroll=UNROLL, wait_late=not UA)
    lax.fori_loop(lo // UNROLL, hi // UNROLL, steps_b, 0)
    if UC:
        steps_c = functools.partial(steps, unroll=UC, do_fwd=False)
        lax.fori_loop(hi // UC, NSEG // UC, steps_c, 0)

    q0 = P0 % RING

    TB = 64
    HB = int(os.environ.get("HB", 64))
    KP = 4

    def combine(n, rows, b):
        g = abg_s[2 * NC + zero, rows, :].astype(f32)
        a = abg_s[n + zero, rows, :].astype(f32)
        if b is None:
            b = abg_s[NC + n + zero, rows, :]
        b = b.astype(f32)
        abg_s[NC + n, rows, :] = (g * a + (1.0 - g) * b).astype(bf16)

    def post_tile(n):
        conv_inverse(NC - 1, n, (NC - 1) & 1)
        piece = 0
        for c in range(BULK // TB):
            r0 = (q0 + c * TB) % RING
            tail = None
            for kp in range(KP):
                hs = range(kp * H // KP, (kp + 1) * H // KP)
                l2 = jnp.concatenate(
                    [o_rings[ring_of(h)[0]][ring_of(h)[1], r0:r0 + TB, :] for h in hs],
                    axis=1)
                w = wo_u[n, hs[0] * DH // 2:(hs[-1] + 1) * DH // 2, :]
                res = jnp.dot(l2, pltpu.bitcast(w, bf16), preferred_element_type=f32)
                tail = res if tail is None else tail + res
                if kp == KP - 1:
                    combine(n, slice(P0 + c * TB, P0 + (c + 1) * TB), tail.astype(bf16))
                elif piece < P0 // HB:
                    abg_s[2 * NC + 1, 0:16, :] = tail[0:16].astype(bf16)
                if piece < P0 // HB:
                    combine(n, slice(piece * HB, (piece + 1) * HB), None)
                    piece += 1
                    if piece == P0 // HB:
                        out_copy(n, 0).start()
        out_copy(n, 1).start()

    def post_body(it, carry):
        for u in range(POSTU):
            post_tile(it * POSTU + u)
        return carry

    lax.fori_loop(0, NC // POSTU, post_body, 0)
    for n in range(NC):
        out_copy(n, 0).wait()
        out_copy(n, 1).wait()


@functools.partial(jax.jit, static_argnames=("B_seg_len",))
def pallas_gated_mix__ssm_conv_h3__memory_aug_recurrent_mem_tr__prompt_kernel(
    A_q: jax.Array,
    A_k: jax.Array,
    A_v: jax.Array,
    A_shift_k: jax.Array,
    A_ssm_k: jax.Array,
    A_ssm_D: jax.Array,
    B_x: jax.Array,
    B_mem0: jax.Array,
    B_Wq: jax.Array,
    B_Wk: jax.Array,
    B_Wv: jax.Array,
    B_Wo: jax.Array,
    B_seg_len,
    gate_w: jax.Array,
):
    del B_x
    assert int(B_seg_len) == SEG
    assert A_q.shape == (1, S, D) and B_Wq.shape == (D, H, DH)
    assert B_mem0.shape == (1, M, D) and A_shift_k.shape == (D, KS)

    n_pre = NB + 4 + 4 + NC + NC
    scratch = [
        pltpu.VMEM((NC, S, 128), bf16),
        pltpu.VMEM((2, NC, S + 2 * PAD, 128), bf16),
        pltpu.VMEM((NB, D, 128), bf16),
        pltpu.VMEM((NC, S, 128), bf16),
        pltpu.VMEM((2 * NC + 2, S, 128), bf16),
        pltpu.VMEM((3 * H // 2, D // 2, 128), u32),
        pltpu.VMEM((3 * H // 2, D // 2, 128), u32),
        pltpu.VMEM((NC, H * DH, 128), bf16),
        pltpu.VMEM((NSLOT, D + 8, HC, 128), bf16),
        pltpu.VMEM((8 * RP * HC // 2, 128), u32),
        pltpu.VMEM((3 * H // 2, RING, 128), bf16),
        pltpu.VMEM((3 * H // 2, RING, 128), bf16),
        pltpu.VMEM((H // 2, RING, 128), bf16),
        pltpu.VMEM((H // 2, RING, 128), bf16),
        pltpu.VMEM((4 * NB + 1, NF, 128), f32),
        pltpu.VMEM((2, NB, NF, 128), bf16),
        pltpu.VMEM((NF, BL), bf16),
        pltpu.VMEM((BL, NF), bf16),
        pltpu.VMEM((H // 2, 2 * LTOT, 2 * LTOT), bf16),
        pltpu.VMEM((NC, TP + M, 128), f32),
        pltpu.VMEM((M, D), bf16),
        pltpu.VMEM((KS, D), bf16),
        pltpu.VMEM((NC, 128), bf16),
        pltpu.VMEM((NC, 128), bf16),
        pltpu.VMEM((NC, KS + 2, 8, 128), f32),
        pltpu.SMEM((1,), jnp.int32),
        pltpu.SemaphoreType.DMA((NSLOT,)),
        pltpu.SemaphoreType.DMA((NC,)),
        pltpu.SemaphoreType.DMA((n_pre,)),
        pltpu.SemaphoreType.DMA((1,)),
        pltpu.SemaphoreType.DMA((2 * NC,)),
    ]
    out = pl.pallas_call(
        _kernel,
        out_shape=jax.ShapeDtypeStruct((S, D), bf16),
        in_specs=[pl.BlockSpec(memory_space=pl.ANY)] * 12,
        out_specs=pl.BlockSpec(memory_space=pl.ANY),
        scratch_shapes=scratch,
        compiler_params=pltpu.CompilerParams(
            vmem_limit_bytes=124 * 1024 * 1024,
            disable_bounds_checks=bool(int(os.environ.get('NOBC', 1))),
            disable_semaphore_checks=bool(int(os.environ.get('NOSC', 1)))),
    )(
        A_q.reshape(S, D), A_k.reshape(S, D), A_v.reshape(S, D),
        A_shift_k.T, A_ssm_k, A_ssm_D.reshape(NC, 128), B_mem0.reshape(M, D),
        B_Wq, B_Wk, B_Wv, B_Wo.reshape(H * DH, D), gate_w.reshape(NC, 128),
    )
    return out.reshape(1, S, D)
```

```python
import functools
import math

import jax
import jax.numpy as jnp
from jax import lax
import jax.experimental.pallas as pl
import jax.experimental.pallas.tpu as pltpu

bf16 = jnp.bfloat16
f32 = jnp.float32
u32 = jnp.uint32

S = 2048
D = 1024
H = 32
DH = 128
M = 8
SEG = 32
NSEG = S // SEG
KS = 4
TP = 24
BULK = S - TP * NSEG
P0 = TP * NSEG
RING = 576
NC = D // 128
BL = 128
NB = S // BL
NF = 2 * BL
G = 8
HC = 8
NCH = 3 * H // HC
PAD = 16
LTOT = SEG + M
NSLOT = 4
RP = 16
KVP = 32
NLAST = 8


def _make_plan():
    plan = {}
    done = 0
    for i in range(60):
        tgt = (i + 1) * 144 // 60
        plan[i] = (tgt - done, 0)
        done = tgt
    for j in range(2 * BL // KVP):
        i = 3 + 12 * j
        plan[i] = (plan.get(i, (0, 0))[0], 1)
    return plan


PLAN = _make_plan()


def _ring(x):
    x = jnp.where(x >= 2 * RING, x - 2 * RING, x)
    return jnp.where(x >= RING, x - RING, x)


def _kernel(x_hbm, k_hbm, v_hbm, shift_hbm, filt_hbm, dvec_hbm, mem0_hbm,
            wq_hbm, wk_hbm, wv_hbm, wo_hbm, gate_hbm,
            out_hbm,
            x_s, kin_s, f_s, kv_s, abg_s,
            w0_s, w1_s, wo_s, stage, qkv0_s, qkv1_s, o0_s, o1_s,
            uk_s, z_s, fw_s, fi_s, p_s, acc_s, qm_s, l2_s,
            mem_s, shift_s, dvec_s, gate_s, prm_s, zero_s,
            sem_w, sem_x0, sem_pre, sem_late, sem_out):
    scale = DH ** (-0.5)
    w_hbms = (wq_hbm, wk_hbm, wv_hbm)
    w_bufs = (w0_s, w1_s)
    qkv_rings = (qkv0_s, qkv1_s)
    o_rings = (o0_s, o1_s)

    def ring_of(h):
        g = h // G
        return g % 2, (g // 2) * G + h % G

    def chunk_group(c):
        return (c % 4) ^ 1 if c // 4 == 2 else c % 4

    def tile_of(m, h):
        c = [c for c in range(4 * m, 4 * m + 4) if chunk_group(c) == h // G][0]
        return c % 2, (c // 2) * HC + h % G

    sem_idx = [0]

    def next_sem():
        sem_idx[0] += 1
        return sem_pre.at[sem_idx[0] - 1]

    def x0_copy(n):
        return pltpu.make_async_copy(
            x_hbm.at[pl.ds(0, BULK), pl.ds(n * 128, 128)],
            x_s.at[n, pl.ds(0, BULK), :], sem_x0.at[n])

    def w_copy(c, slot):
        return pltpu.make_async_copy(
            w_hbms[c // 4].at[:, pl.ds(chunk_group(c) * HC, HC), :],
            stage.at[slot, pl.ds(0, D)], sem_w.at[slot])

    def kv_copies(n, sem_k, sem_v):
        return [
            pltpu.make_async_copy(k_hbm.at[:, pl.ds(n * 128, 128)],
                                  kin_s.at[0, n, pl.ds(PAD, S), :], sem_k),
            pltpu.make_async_copy(v_hbm.at[:, pl.ds(n * 128, 128)],
                                  kin_s.at[1, n, pl.ds(PAD, S), :], sem_v),
        ]

    def filt_copy(d):
        return pltpu.make_async_copy(filt_hbm.at[:, pl.ds(d * 128, 128)],
                                     f_s.at[d], next_sem())

    def xrest_copy(n):
        return pltpu.make_async_copy(
            x_hbm.at[pl.ds(BULK, S - BULK), pl.ds(n * 128, 128)],
            x_s.at[n, pl.ds(BULK, S - BULK), :], next_sem())

    def wo_copy(n):
        return pltpu.make_async_copy(wo_hbm.at[:, pl.ds(n * 128, 128)],
                                     wo_s.at[n], next_sem())

    conv_groups = [
        [filt_copy(d) for d in range(0, NB // 2)],
        [filt_copy(d) for d in range(NB // 2, NB)],
        kv_copies(0, next_sem(), next_sem()) + kv_copies(1, next_sem(), next_sem()) + [
            pltpu.make_async_copy(mem0_hbm, mem_s, next_sem()),
            pltpu.make_async_copy(shift_hbm, shift_s.at[0], next_sem()),
            pltpu.make_async_copy(dvec_hbm, dvec_s.at[0], next_sem()),
            pltpu.make_async_copy(gate_hbm, gate_s.at[0], next_sem()),
        ],
    ]
    main_groups = [
        [xrest_copy(n) for n in range(0, NC // 2)],
        [xrest_copy(n) for n in range(NC // 2, NC)],
    ] + [[wo_copy(2 * q), wo_copy(2 * q + 1)] for q in range(4)]
    pre_groups = conv_groups + main_groups
    late = []
    for n in range(2, NC):
        late += kv_copies(n, sem_late.at[0], sem_late.at[0])
    late_dst = kin_s.at[:, pl.ds(2, NC - 2), pl.ds(PAD, S), :]
    late_all = pltpu.make_async_copy(late_dst, late_dst, sem_late.at[0])

    def out_copy(n, tail):
        rows = pl.ds(P0, S - P0) if tail else pl.ds(0, P0)
        return pltpu.make_async_copy(abg_s.at[NC + n, rows, :],
                                     out_hbm.at[rows, pl.ds(n * 128, 128)],
                                     sem_out.at[2 * n + tail])

    def dft_table(shape, rho_axis, row0):
        row = lax.broadcasted_iota(jnp.int32, shape, 0) + row0
        col = lax.broadcasted_iota(jnp.int32, shape, 1)
        rho, t = (row, col) if rho_axis == 0 else (col, row)
        f = ((rho >> 5) << 4) + ((rho & 7) << 1) + ((rho >> 3) & 1)
        im = (rho >> 4) & 1
        ph = ((2 * f + 1) * t + im * BL) & (4 * BL - 1)
        ph = jnp.where(ph > 2 * BL, 4 * BL - ph, ph)
        return jnp.cos(ph.astype(f32) * (math.pi / NF))

    def fw_body(i, carry):
        r0 = pl.multiple_of(i * (NF // 4), NF // 4)
        fw_s[pl.ds(r0, NF // 4), :] = dft_table((NF // 4, BL), 0, r0).astype(bf16)
        for n in range(2):
            kin_s[0, 2 * i + n, 0:PAD, :] = jnp.zeros((PAD, 128), bf16)
        return carry

    def fi_body(i, carry):
        r0 = pl.multiple_of(i * (BL // 4), BL // 4)
        tab = (dft_table((BL // 4, NF), 1, r0) * (1.0 / BL)).astype(bf16)
        fi_s[0, pl.ds(r0, BL // 4), :] = tab[:, :BL]
        fi_s[1, pl.ds(r0, BL // 4), :] = tab[:, BL:]
        for n in range(NB // 4):
            z_s[1, (NB // 4) * i + n] = jnp.zeros((NF, 128), bf16)
        return carry

    w_copy(0, 0).start()
    zero_s[0] = 0
    lax.fori_loop(0, 4, fw_body, 0)
    for n in range(NC):
        x0_copy(n).start()
    lax.fori_loop(0, 4, fi_body, 0)
    w_copy(1, 1).start()
    zero = zero_s[0]

    def conv_filter_dft(ct, d, slot):
        c0 = ct * 128 if isinstance(ct, int) else pl.multiple_of(ct * 128, 128)
        uk_s[(2 * slot + 1) * NB + d] = lax.dot_general(
            fw_s[...], f_s[d, pl.ds(c0, 128), :], (((1,), (1,)), ((), ())),
            preferred_element_type=f32)

    def conv_kv(ct, row0):
        kk = kin_s[0, ct, pl.ds(row0, KVP + PAD), :].astype(f32)
        ks = kk[PAD:] * prm_s[ct, 0, 0:1, :]
        for tau in range(1, KS):
            ks = ks + kk[PAD - tau:KVP + PAD - tau] * prm_s[ct, tau, 0:1, :]
        vv = kin_s[1, ct, pl.ds(row0 + PAD, KVP), :].astype(f32)
        kv_s[ct, pl.ds(row0, KVP), :] = (ks * vv).astype(bf16)

    def kv_anchor(pos, val):
        kin_s[0, 0, pl.ds(S + PAD + pos, 8), :] = val

    def conv_kv_dft(ct, j, slot):
        r0 = j * BL if isinstance(j, int) else pl.multiple_of(j * BL, BL)
        uk_s[2 * slot * NB + j] = jnp.dot(
            fw_s[...], kv_s[ct, pl.ds(r0, BL), :], preferred_element_type=f32)

    def conv_products(r, slot):
        ub = 2 * slot * NB
        kb = ub + NB

        def cmac(acc, k, u):
            pr = k[0] * u[0] - k[1] * u[1]
            pi = k[0] * u[1] + k[1] * u[0]
            return (pr, pi) if acc is None else (acc[0] + pr, acc[1] + pi)

        for par in range(2):
            ore = pl.multiple_of(r * 32, 32) + 8 * par
            oim = pl.multiple_of(r * 32, 32) + (16 + 8 * par)

            def load(idx):
                return (uk_s[idx, pl.ds(ore, 8), :], uk_s[idx, pl.ds(oim, 8), :])

            prev = None
            for i in range(0, NB, 2):
                y0 = y1 = None
                khi = load(kb + i + 1)
                for j in range(i + 2):
                    u = load(ub + j)
                    y1 = cmac(y1, khi, u)
                    if j <= i:
                        khi = load(kb + i - j)
                        y0 = cmac(y0, khi, u)
                    if j < i + 1:
                        yield
                for ii, y in ((i, y0), (i + 1, y1)):
                    if prev is None:
                        zr, zi = y
                    elif par == 0:
                        zr, zi = y[0] - prev[1], y[1] + prev[0]
                    else:
                        zr, zi = y[0] + prev[1], y[1] - prev[0]
                    prev = y
                    z_s[slot, ii, pl.ds(ore, 8), :] = zr.astype(bf16)
                    z_s[slot, ii, pl.ds(oim, 8), :] = zi.astype(bf16)
                yield

    def conv_inverse(ct, r, slot):
        dvec = prm_s[ct, KS, 0:1, :]
        for jj in range(2):
            i = 2 * r + jj
            r0 = pl.multiple_of(i * BL, BL)
            fi = jnp.concatenate([fi_s[0], fi_s[1]], axis=1)
            y = jnp.dot(fi, z_s[slot, i], preferred_element_type=f32)
            y = y + kv_s[ct, pl.ds(r0, BL), :].astype(f32) * dvec
            a = x_s[ct, pl.ds(r0, BL), :].astype(f32) * y
            abg_s[ct, pl.ds(r0, BL), :] = a.astype(bf16)

    NPIECE = D // RP

    def transpose4(v):
        sub = lax.broadcasted_iota(jnp.int32, (8, 128), 0)
        v = list(v)
        for s in (2, 1):
            keep = (sub & s) == 0
            for q in range(4):
                if not q & s:
                    a, b = v[q], v[q + s]
                    v[q] = jnp.where(keep, a, pltpu.roll(b, s, 0))
                    v[q + s] = jnp.where(keep, pltpu.roll(a, 8 - s, 0), b)
        return v

    def relayout(par, half, slot, p):
        def two_tiles(d):
            t = jnp.stack([stage[slot, d], stage[slot, d + RP // 2]])
            return pltpu.bitcast(t.reshape(2 * HC, 128), u32)

        lo, hi = [], []
        for q in range(4):
            ev = two_tiles(p * RP + 2 * q)
            od = two_tiles(p * RP + 2 * q + 1)
            lo.append((ev & jnp.uint32(0xFFFF)) | (od << 16))
            hi.append((ev >> 16) | (od & jnp.uint32(0xFFFF0000)))
        lo = transpose4(lo)
        hi = transpose4(hi)
        r0 = p * (RP // 2)
        rows = pl.ds(r0 if isinstance(p, int) else pl.multiple_of(r0, RP // 2), RP // 2)
        for j in range(HC // 2):
            w_bufs[par][half * HC + 2 * j, rows, :] = lo[j]
            w_bufs[par][half * HC + 2 * j + 1, rows, :] = hi[j]

    def wtile(m, h):
        par, t = tile_of(m, h)
        return pltpu.bitcast(w_bufs[par][t], bf16)

    x_u = x_s.bitcast(u32)

    def bulk_dot(par, half, hh):
        xb = jnp.concatenate(
            [pltpu.bitcast(x_u[t, 0:BULK // 2, :], bf16) for t in range(NC)], axis=1)
        w = pltpu.bitcast(w_bufs[par][half * HC + hh], bf16)
        r = jnp.dot(xb, w, preferred_element_type=f32).astype(bf16)
        qkv_rings[par][half * HC + hh, 0:BULK, :] = r
        return r

    def start_copies(cond):
        def start(pred, make):
            def go():
                for c in make():
                    c.start()
            if pred is True:
                go()
            elif pred is not False:
                pl.when(pred)(go)

        for c in range(NCH - NSLOT):
            start(cond(c), lambda: [w_copy(c + NSLOT, c % NSLOT)])
        for gi, group in enumerate(pre_groups):
            start(cond(gi + 2), lambda: group)

    def chunk_dots(par, half, aslot, nhalf, nslot, first):
        for hh in range(HC):
            if hh == first and first > 0:
                w_copy(0, nslot).wait()
            r = bulk_dot(par, half, hh)
            if hh >= first:
                p0 = (hh - first) * NPIECE // (HC - first)
                p1 = (hh - first + 1) * NPIECE // (HC - first)
                for p in range(p0, p1):
                    q0 = ((p - p0) * (BULK // HC) // (p1 - p0)) * HC
                    stage[aslot, D] = r[q0:q0 + HC]
                    relayout(1 - par, nhalf, nslot, p)

    w_copy(0, 0).wait()
    w_copy(2, 2).start()

    def relayout0(i, carry):
        for q in range(8):
            relayout(0, 0, 0, i * 8 + q)
        return carry

    lax.fori_loop(0, NPIECE // 8, relayout0, 0)
    for n in range(NC):
        x0_copy(n).wait()
        if n == 0:
            w_copy(3, 3).start()
    start_copies(lambda c: c == 0)
    chunk_dots(0, 0, zero, 0, 1, 4)

    def pre_body(k, carry):
        for par in (1, 0):
            i = 2 * k + 2 - par
            nslot = (i + 1) % NSLOT
            w_copy(0, nslot).wait()
            start_copies(lambda c: (i == c) if (c % 2 == par and c > 0) else False)
            chunk_dots(par, k + 1 - par, i % NSLOT, k + 1, nslot, 0)
        return carry

    lax.fori_loop(0, NCH // 2 - 1, pre_body, 0)

    for group in conv_groups:
        for c in group:
            c.wait()
    for c in late:
        c.start()
    taps = shift_s[0].astype(f32)
    dv = dvec_s[0].astype(f32)
    gw = gate_s[0].astype(f32)
    for n in range(NC):
        for tau in range(KS):
            prm_s[n, tau] = jnp.broadcast_to(
                taps[tau:tau + 1, n * 128:(n + 1) * 128], (8, 128))
        prm_s[n, KS] = jnp.broadcast_to(dv[n:n + 1], (8, 128))
        prm_s[n, KS + 1] = jnp.broadcast_to(gw[n:n + 1], (8, 128))

    zpos = pl.multiple_of(zero * 8, 8)
    for hh in range(HC):
        r = bulk_dot(1, NCH // 2 - 1, hh)
        for q in range(2 * BL // KVP):
            kv_anchor(zpos, r[q * KVP * 2:q * KVP * 2 + 8])
            conv_kv(0, 2 * BL * hh + KVP * q)
            if q == 0:
                conv_kv(1, KVP * hh)
        for d in (2 * hh, 2 * hh + 1):
            conv_filter_dft(0, d, 0)
        if hh > 0:
            for j in (2 * hh - 2, 2 * hh - 1):
                conv_kv_dft(0, j, 0)
    for j in (NB - 2, NB - 1):
        conv_kv_dft(0, j, 0)
    for group in main_groups:
        for c in group:
            c.wait()

    wo_u = wo_s.bitcast(u32)

    def attn_mask():
        row = lax.broadcasted_iota(jnp.int32, (2 * LTOT, 2 * LTOT), 0)
        col = lax.broadcasted_iota(jnp.int32, (2 * LTOT, 2 * LTOT), 1)
        row_mem = row >= 2 * SEG
        col_mem = col >= 2 * SEG
        row_head = jnp.where(row_mem, (row - 2 * SEG) // M, row // SEG)
        col_head = jnp.where(col_mem, (col - 2 * SEG) // M, col // SEG)
        same = row_head == col_head
        mask = same & (row_mem | col_mem | (col <= row))
        fill = jnp.where(same, -1e9 / scale, -jnp.inf).astype(f32)
        return mask, fill

    ring_u = tuple(r.bitcast(u32) for r in qkv_rings)

    def step(s, mem, do_fwd, odd):
        mask, fill = attn_mask()

        ct = s >> 3
        r = s & 7
        cnext = jnp.minimum(ct + 1, NC - 1)
        cprev = jnp.maximum(ct - 1, 0)
        slot = ct & 1
        oslot = 1 - slot

        o16, o8 = (8, 0) if odd else (0, 16)
        al = 8 if odd is None else 16

        def pieces(base, wrap):
            f = _ring if wrap else (lambda v: v)
            if odd is None:
                return [(pl.multiple_of(f(base + 8 * j), 8), 8) for j in range(3)]
            return [(pl.multiple_of(f(base + o16), 16), 16),
                    (pl.multiple_of(f(base + o8), 8), 8)]

        xpos = pieces(BULK + TP * s, False)
        wpos = pieces(BULK + TP * s, True)
        bpos = pieces(TP * s, False)
        rpos = pl.multiple_of(_ring(SEG * s), SEG)
        l16 = pl.multiple_of(_ring(TP * s + o16), al)
        l8 = pl.multiple_of(_ring(TP * s + o8), 8)

        def store_rows(ref, lead, pos, val):
            r0 = 0
            for p0, n in pos:
                ref[lead, pl.ds(p0, n), :] = val[r0:r0 + n]
                r0 += n

        rhalf = pl.multiple_of(rpos >> 1, SEG // 2)
        gpos = pl.multiple_of(SEG * s, SEG)
        apos = pl.multiple_of(r * 8, 8)
        kpos = pl.multiple_of((r & 1) * 8, 8)

        lhs = jnp.concatenate(
            [jnp.concatenate([x_s[t, pl.ds(p0, n), :] for t in range(NC)], axis=1)
             for p0, n in xpos] + [mem], axis=0)

        rls = [None] * H
        acc = [None] * NC

        prods = conv_products(r, slot)
        ckv = jnp.minimum(((s + 1) >> 3) + 1, NC - 1)
        kv_rows = [pl.multiple_of(((s + 1) & 7) * 2 * BL + q * KVP, KVP)
                   for q in range(2 * BL // KVP)] if do_fwd else []

        def release(key, res):
            n_prod, n_kv = PLAN.get(key, (0, 0))
            if n_prod:
                uk_s[4 * NB, pl.ds(apos, 8), :] = res[0:8]
                for _ in range(n_prod):
                    next(prods, None)
            if n_kv and kv_rows:
                kv_anchor(kpos, res[0:8].astype(bf16))
                conv_kv(ckv, kv_rows.pop(0))

        n_dot = [0]

        def proj(m, h):
            ri, t = tile_of(m, h)
            res = jnp.dot(lhs, wtile(m, h), preferred_element_type=f32)
            release(n_dot[0], res)
            n_dot[0] += 1
            res = res.astype(bf16)
            store_rows(qkv_rings[ri], t, wpos, res)
            qm_s[m * (H // 2) + h // 2, (h % 2) * M:(h % 2 + 1) * M, :] = res[TP:]

        def pair_rows(m, h):
            ri, t = tile_of(m, h)
            tok = [pltpu.bitcast(ring_u[ri][t + i, pl.ds(rhalf, SEG // 2), :], bf16)
                   for i in range(2)]
            return jnp.concatenate(tok + [qm_s[m * (H // 2) + h // 2]], axis=0)

        def att_qk(h):
            sc = lax.dot_general(pair_rows(0, h), pair_rows(1, h),
                                 (((1,), (1,)), ((), ())), preferred_element_type=f32)
            sc = jnp.where(mask, sc, fill)
            mx = jnp.max(sc, axis=-1, keepdims=True)
            p = jnp.exp2((sc - mx) * (scale * math.log2(math.e)))
            den = jnp.sum(p, axis=-1, keepdims=True)
            rl = pl.reciprocal(den, approx=True)
            rls[h] = rl * (2.0 - den * rl)
            p_s[h // 2] = p.astype(bf16)

        def att_pv(h):
            ri, t = ring_of(h)
            o = jnp.dot(p_s[h // 2], pair_rows(2, h), preferred_element_type=f32)
            o = (o * rls[h]).astype(bf16)
            for i in range(2):
                o_rings[ri][t + i, pl.ds(rpos, SEG), :] = o[i * SEG:(i + 1) * SEG]
            for i in range(2):
                l2_s[h + i, M:, :] = o[2 * SEG + i * M:2 * SEG + (i + 1) * M]
            for i in range(2):
                l2_s[h + i, 0:M, :] = o_rings[ri][t + i, pl.ds(l8, M), :]

        def wo_grp(g):
            h0 = g * G
            parts = []
            for h in range(h0, h0 + G):
                ri, t = ring_of(h)
                parts.append(jnp.concatenate(
                    [o_rings[ri][t, pl.ds(l16, 16), :], l2_s[h]], axis=0))
            l2 = jnp.concatenate(parts, axis=1)
            for n in range(NC):
                w = pltpu.bitcast(wo_u[n, h0 * DH // 2:(h0 + G) * DH // 2, :], bf16)
                res = jnp.dot(l2, w, preferred_element_type=f32)
                if g == 0:
                    acc_s[n] = res
                else:
                    acc[n] = (acc_s[n] if g == 1 else acc[n]) + res

        def gate():
            tot = None
            for n in range(NC):
                xv = x_s[n, pl.ds(gpos, SEG), :].astype(f32) * prm_s[n, KS + 1, 0:1, :]
                tot = xv if tot is None else tot + xv
            z = jnp.sum(tot, axis=-1, keepdims=True)
            abg_s[2 * NC, pl.ds(gpos, SEG), :] = jnp.broadcast_to(
                jax.nn.sigmoid(z), (SEG, 128)).astype(bf16)

        def qkv_grp(g):
            heads = range(g * G, (g + 1) * G)
            for h in heads:
                proj(2, h)
            for h in heads:
                proj(0, h)
                proj(1, h)

        def qk_grp(g):
            for h in range(g * G, (g + 1) * G, 2):
                att_qk(h)

        def pv_grp(g):
            for h in range(g * G, (g + 1) * G, 2):
                att_pv(h)

        conv_inverse(cprev, r, oslot)
        if do_fwd:
            for jj in range(2):
                conv_filter_dft(cnext, 2 * r + jj, oslot)
            for jj in range(2):
                conv_kv_dft(cnext, 2 * r + jj, oslot)
        qkv_grp(0)
        qkv_grp(1)
        qk_grp(0)
        qkv_grp(2)
        pv_grp(0)
        qk_grp(1)
        qkv_grp(3)
        gate()
        pv_grp(1)
        qk_grp(2)
        wo_grp(0)
        pv_grp(2)
        qk_grp(3)
        wo_grp(1)
        pv_grp(3)
        wo_grp(2)
        wo_grp(3)
        for _ in prods:
            pass
        assert not kv_rows
        new_mem = []
        for n in range(NC):
            res = acc[n].astype(bf16)
            store_rows(abg_s, NC + n, bpos, res)
            new_mem.append(res[TP:])
        return jnp.concatenate(new_mem, axis=1)

    def step_pair(it, carry):
        @pl.when(it == 3)
        def _():
            late_all.wait()

        mem = step(2 * it, mem_s[...], True, 0)
        mem_s[...] = step(2 * it + 1, mem, True, 1)
        return carry

    def step_last(s, carry):
        mem_s[...] = step(s, mem_s[...], False, None)
        return carry

    lax.fori_loop(0, (NSEG - NLAST) // 2, step_pair, 0)
    lax.fori_loop(NSEG - NLAST, NSEG, step_last, 0)

    q0 = P0 % RING

    TB = 64
    HB = 64
    KP = 4

    def combine(n, rows, b):
        g = abg_s[2 * NC + zero, rows, :].astype(f32)
        a = abg_s[n + zero, rows, :].astype(f32)
        if b is None:
            b = abg_s[NC + n + zero, rows, :]
        b = b.astype(f32)
        abg_s[NC + n, rows, :] = (g * a + (1.0 - g) * b).astype(bf16)

    def post_tile(n):
        conv_inverse(NC - 1, n, (NC - 1) & 1)
        piece = 0
        for c in range(BULK // TB):
            r0 = (q0 + c * TB) % RING
            tail = None
            for kp in range(KP):
                hs = range(kp * H // KP, (kp + 1) * H // KP)
                l2 = jnp.concatenate(
                    [o_rings[ring_of(h)[0]][ring_of(h)[1], r0:r0 + TB, :] for h in hs],
                    axis=1)
                w = wo_u[n, hs[0] * DH // 2:(hs[-1] + 1) * DH // 2, :]
                res = jnp.dot(l2, pltpu.bitcast(w, bf16), preferred_element_type=f32)
                tail = res if tail is None else tail + res
                if kp == KP - 1:
                    combine(n, slice(P0 + c * TB, P0 + (c + 1) * TB), tail.astype(bf16))
                elif piece < P0 // HB:
                    abg_s[2 * NC + 1, 0:16, :] = tail[0:16].astype(bf16)
                if piece < P0 // HB:
                    combine(n, slice(piece * HB, (piece + 1) * HB), None)
                    piece += 1
                    if piece == P0 // HB:
                        out_copy(n, 0).start()
        out_copy(n, 1).start()

    def post_body(it, carry):
        post_tile(2 * it)
        post_tile(2 * it + 1)
        return carry

    lax.fori_loop(0, NC // 2, post_body, 0)
    for n in range(NC):
        out_copy(n, 0).wait()
        out_copy(n, 1).wait()


@functools.partial(jax.jit, static_argnames=("B_seg_len",))
def pallas_gated_mix__ssm_conv_h3__memory_aug_recurrent_mem_tr__prompt_kernel(
    A_q: jax.Array,
    A_k: jax.Array,
    A_v: jax.Array,
    A_shift_k: jax.Array,
    A_ssm_k: jax.Array,
    A_ssm_D: jax.Array,
    B_x: jax.Array,
    B_mem0: jax.Array,
    B_Wq: jax.Array,
    B_Wk: jax.Array,
    B_Wv: jax.Array,
    B_Wo: jax.Array,
    B_seg_len,
    gate_w: jax.Array,
):
    del B_x
    assert int(B_seg_len) == SEG
    assert A_q.shape == (1, S, D) and B_Wq.shape == (D, H, DH)
    assert B_mem0.shape == (1, M, D) and A_shift_k.shape == (D, KS)

    n_pre = NB + 4 + 4 + NC + NC
    scratch = [
        pltpu.VMEM((NC, S, 128), bf16),
        pltpu.VMEM((2, NC, S + 2 * PAD, 128), bf16),
        pltpu.VMEM((NB, D, 128), bf16),
        pltpu.VMEM((NC, S, 128), bf16),
        pltpu.VMEM((2 * NC + 2, S, 128), bf16),
        pltpu.VMEM((3 * H // 2, D // 2, 128), u32),
        pltpu.VMEM((3 * H // 2, D // 2, 128), u32),
        pltpu.VMEM((NC, H * DH, 128), bf16),
        pltpu.VMEM((NSLOT, D + 8, HC, 128), bf16),
        pltpu.VMEM((3 * H // 2, RING, 128), bf16),
        pltpu.VMEM((3 * H // 2, RING, 128), bf16),
        pltpu.VMEM((H // 2, RING, 128), bf16),
        pltpu.VMEM((H // 2, RING, 128), bf16),
        pltpu.VMEM((4 * NB + 1, NF, 128), f32),
        pltpu.VMEM((2, NB, NF, 128), bf16),
        pltpu.VMEM((NF, BL), bf16),
        pltpu.VMEM((2, BL, BL), bf16),
        pltpu.VMEM((H // 2, 2 * LTOT, 2 * LTOT), bf16),
        pltpu.VMEM((NC, TP + M, 128), f32),
        pltpu.VMEM((3 * H // 2, 2 * M, 128), bf16),
        pltpu.VMEM((H, 2 * M, 128), bf16),
        pltpu.VMEM((M, D), bf16),
        pltpu.VMEM((2, KS, D), bf16),
        pltpu.VMEM((8, NC, 128), bf16),
        pltpu.VMEM((8, NC, 128), bf16),
        pltpu.VMEM((NC, KS + 2, 8, 128), f32),
        pltpu.SMEM((1,), jnp.int32),
        pltpu.SemaphoreType.DMA((NSLOT,)),
        pltpu.SemaphoreType.DMA((NC,)),
        pltpu.SemaphoreType.DMA((n_pre,)),
        pltpu.SemaphoreType.DMA((1,)),
        pltpu.SemaphoreType.DMA((2 * NC,)),
    ]
    out = pl.pallas_call(
        _kernel,
        out_shape=jax.ShapeDtypeStruct((S, D), bf16),
        in_specs=[pl.BlockSpec(memory_space=pl.ANY)] * 12,
        out_specs=pl.BlockSpec(memory_space=pl.ANY),
        scratch_shapes=scratch,
        compiler_params=pltpu.CompilerParams(
            vmem_limit_bytes=124 * 1024 * 1024,
            disable_bounds_checks=True,
            disable_semaphore_checks=True),
    )(
        A_q.reshape(S, D), A_k.reshape(S, D), A_v.reshape(S, D),
        A_shift_k.T, A_ssm_k, A_ssm_D.reshape(NC, 128), B_mem0.reshape(M, D),
        B_Wq, B_Wk, B_Wv, B_Wo.reshape(H * DH, D), gate_w.reshape(NC, 128),
    )
    return out.reshape(1, S, D)
```

```python
import math

import jax
import jax.numpy as jnp
from jax import lax
import jax.experimental.pallas as pl
import jax.experimental.pallas.tpu as pltpu

bf16 = jnp.bfloat16
f32 = jnp.float32
u32 = jnp.uint32

S = 2048
D = 1024
H = 32
DH = 128
M = 8
SEG = 32
NSEG = S // SEG
KS = 4
TP = 24
BULK = S - TP * NSEG
P0 = TP * NSEG
RING = 576
NC = D // 128
BL = 128
NB = S // BL
NF = 2 * BL
G = 8
HC = 8
NCH = 3 * H // HC
PAD = 16
LTOT = SEG + M
NSLOT = 4
RP = 16
KVP = 32
NLAST = 8


def _make_plan():
    plan = {}
    done = 0
    for i in range(60):
        tgt = (i + 1) * 144 // 60
        plan[i] = (tgt - done, 0)
        done = tgt
    for j in range(2 * BL // KVP):
        i = 3 + 12 * j
        plan[i] = (plan.get(i, (0, 0))[0], 1)
    return plan


PLAN = _make_plan()


def _ring(x):
    x = jnp.where(x >= 2 * RING, x - 2 * RING, x)
    return jnp.where(x >= RING, x - RING, x)


def _kernel(x_hbm, k_hbm, v_hbm, shift_hbm, filt_hbm, dvec_hbm, mem0_hbm,
            wq_hbm, wk_hbm, wv_hbm, wo_hbm, gate_hbm,
            out_hbm,
            x_s, xb_s, kin_s, f_s, kv_s, abg_s,
            w0_s, w1_s, wo_s, wo_u, stage, qkv0_s, qkv1_s, o0_s, o1_s,
            uk_s, z_s, fw_s, fi_s, p_s, acc_s, qm_s, l2_s,
            mem_s, shift_s, dvec_s, gate_s, prm_s, zero_s,
            sem_w, sem_x0, sem_wo, sem_pre, sem_late, sem_out):
    scale = DH ** (-0.5)
    w_hbms = (wq_hbm, wk_hbm, wv_hbm)
    w_bufs = (w0_s, w1_s)
    qkv_rings = (qkv0_s, qkv1_s)
    o_rings = (o0_s, o1_s)

    def ring_of(h):
        g = h // G
        return g % 2, (g // 2) * G + h % G

    def chunk_group(c):
        return (c % 4) ^ 1 if c // 4 == 2 else c % 4

    def tile_of(m, h):
        c = [c for c in range(4 * m, 4 * m + 4) if chunk_group(c) == h // G][0]
        return c % 2, (c // 2) * HC + h % G

    sem_idx = [0]

    def next_sem():
        sem_idx[0] += 1
        return sem_pre.at[sem_idx[0] - 1]

    def x0_copy(n):
        return pltpu.make_async_copy(
            x_hbm.at[pl.ds(0, BULK), pl.ds(n * 128, 128)],
            x_s.at[n, pl.ds(0, BULK), :], sem_x0.at[n])

    def w_copy(c, slot):
        return pltpu.make_async_copy(
            w_hbms[c // 4].at[:, pl.ds(chunk_group(c) * HC, HC), :],
            stage.at[slot, pl.ds(0, D)], sem_w.at[slot])

    def kv_copies(n, sem_k, sem_v):
        return [
            pltpu.make_async_copy(k_hbm.at[:, pl.ds(n * 128, 128)],
                                  kin_s.at[0, n, pl.ds(PAD, S), :], sem_k),
            pltpu.make_async_copy(v_hbm.at[:, pl.ds(n * 128, 128)],
                                  kin_s.at[1, n, pl.ds(PAD, S), :], sem_v),
        ]

    def filt_copy(d):
        return pltpu.make_async_copy(filt_hbm.at[:, pl.ds(d * 128, 128)],
                                     f_s.at[d], next_sem())

    def xrest_copy(n):
        return pltpu.make_async_copy(
            x_hbm.at[pl.ds(BULK, S - BULK), pl.ds(n * 128, 128)],
            x_s.at[n, pl.ds(BULK, S - BULK), :], next_sem())

    def wo_copy(n, src_n=None):
        src_n = n if src_n is None else src_n
        return pltpu.make_async_copy(wo_hbm.at[:, pl.ds(src_n * 128, 128)],
                                     wo_s.at[n, pl.ds(0, H * DH), :], sem_wo.at[n])

    conv_groups = [[filt_copy(d) for d in range(4 * q, 4 * q + 4)] for q in range(4)] + [
        kv_copies(0, next_sem(), next_sem()) + [
            pltpu.make_async_copy(mem0_hbm, mem_s, next_sem()),
            pltpu.make_async_copy(shift_hbm, shift_s.at[0], next_sem()),
            pltpu.make_async_copy(dvec_hbm, dvec_s.at[0], next_sem()),
            pltpu.make_async_copy(gate_hbm, gate_s.at[0], next_sem()),
        ],
        kv_copies(1, next_sem(), next_sem()),
    ]
    main_groups = [
        [xrest_copy(n) for n in range(0, NC // 2)],
        [xrest_copy(n) for n in range(NC // 2, NC)],
    ]
    pre_groups = conv_groups + main_groups
    late = []
    for n in range(2, NC):
        late += kv_copies(n, sem_late.at[0], sem_late.at[0])
    late_dst = kin_s.at[:, pl.ds(2, NC - 2), pl.ds(PAD, S), :]
    late_all = pltpu.make_async_copy(late_dst, late_dst, sem_late.at[0])

    def out_copy(n, tail):
        rows = pl.ds(P0, S - P0) if tail else pl.ds(0, P0)
        return pltpu.make_async_copy(abg_s.at[NC + n, rows, :],
                                     out_hbm.at[rows, pl.ds(n * 128, 128)],
                                     sem_out.at[2 * n + tail])

    def dft_table(shape, rho_axis, row0):
        row = lax.broadcasted_iota(jnp.int32, shape, 0) + row0
        col = lax.broadcasted_iota(jnp.int32, shape, 1)
        rho, t = (row, col) if rho_axis == 0 else (col, row)
        f = ((rho >> 5) << 4) + ((rho & 7) << 1) + ((rho >> 3) & 1)
        im = (rho >> 4) & 1
        ph = ((2 * f + 1) * t + im * BL) & (4 * BL - 1)
        ph = jnp.where(ph > 2 * BL, 4 * BL - ph, ph)
        return jnp.cos(ph.astype(f32) * (math.pi / NF))

    def fw_body(i, carry):
        r0 = pl.multiple_of(i * (NF // 4), NF // 4)
        fw_s[pl.ds(r0, NF // 4), :] = dft_table((NF // 4, BL), 0, r0).astype(bf16)
        for n in range(2):
            kin_s[0, 2 * i + n, 0:PAD, :] = jnp.zeros((PAD, 128), bf16)
        q0 = pl.multiple_of(i * (H * DH // 4), H * DH // 4)
        wo_s[NC, pl.ds(q0, H * DH // 4), :] = jnp.zeros((H * DH // 4, 128), bf16)
        return carry

    def fi_body(i, carry):
        r0 = pl.multiple_of(i * (BL // 4), BL // 4)
        tab = (dft_table((BL // 4, NF), 1, r0) * (1.0 / BL)).astype(bf16)
        fi_s[0, pl.ds(r0, BL // 4), :] = tab[:, :BL]
        fi_s[1, pl.ds(r0, BL // 4), :] = tab[:, BL:]
        for n in range(NB // 4):
            z_s[1, (NB // 4) * i + n] = jnp.zeros((NF, 128), bf16)
        return carry

    w_copy(0, 0).start()
    zero_s[0] = 0
    lax.fori_loop(0, 4, fw_body, 0)
    for n in range(NC):
        x0_copy(n).start()
    lax.fori_loop(0, 4, fi_body, 0)
    w_copy(1, 1).start()
    zero = zero_s[0]

    def conv_filter_dft(ct, d, slot):
        c0 = ct * 128 if isinstance(ct, int) else pl.multiple_of(ct * 128, 128)
        uk_s[(2 * slot + 1) * NB + d] = lax.dot_general(
            fw_s[...], f_s[d, pl.ds(c0, 128), :], (((1,), (1,)), ((), ())),
            preferred_element_type=f32)

    def conv_kv(ct, row0):
        kk = kin_s[0, ct, pl.ds(row0, KVP + PAD), :].astype(f32)
        ks = kk[PAD:] * prm_s[ct, 0, 0:1, :]
        for tau in range(1, KS):
            ks = ks + kk[PAD - tau:KVP + PAD - tau] * prm_s[ct, tau, 0:1, :]
        vv = kin_s[1, ct, pl.ds(row0 + PAD, KVP), :].astype(f32)
        kv_s[ct, pl.ds(row0, KVP), :] = (ks * vv).astype(bf16)

    def kv_anchor(pos, val):
        kin_s[0, 0, pl.ds(S + PAD + pos, 8), :] = val

    def conv_kv_dft(ct, j, slot):
        r0 = j * BL if isinstance(j, int) else pl.multiple_of(j * BL, BL)
        uk_s[2 * slot * NB + j] = jnp.dot(
            fw_s[...], kv_s[ct, pl.ds(r0, BL), :], preferred_element_type=f32)

    def conv_products(r, slot):
        ub = 2 * slot * NB
        kb = ub + NB

        def cmac(acc, k, u):
            pr = k[0] * u[0] - k[1] * u[1]
            pi = k[0] * u[1] + k[1] * u[0]
            return (pr, pi) if acc is None else (acc[0] + pr, acc[1] + pi)

        for par in range(2):
            ore = pl.multiple_of(r * 32, 32) + 8 * par
            oim = pl.multiple_of(r * 32, 32) + (16 + 8 * par)

            def load(idx):
                return (uk_s[idx, pl.ds(ore, 8), :], uk_s[idx, pl.ds(oim, 8), :])

            prev = None
            for i in range(0, NB, 2):
                y0 = y1 = None
                khi = load(kb + i + 1)
                for j in range(i + 2):
                    u = load(ub + j)
                    y1 = cmac(y1, khi, u)
                    if j <= i:
                        khi = load(kb + i - j)
                        y0 = cmac(y0, khi, u)
                    if j < i + 1:
                        yield
                for ii, y in ((i, y0), (i + 1, y1)):
                    if prev is None:
                        zr, zi = y
                    elif par == 0:
                        zr, zi = y[0] - prev[1], y[1] + prev[0]
                    else:
                        zr, zi = y[0] + prev[1], y[1] - prev[0]
                    prev = y
                    z_s[slot, ii, pl.ds(ore, 8), :] = zr.astype(bf16)
                    z_s[slot, ii, pl.ds(oim, 8), :] = zi.astype(bf16)
                yield

    def conv_inverse(ct, r, slot):
        dvec = prm_s[ct, KS, 0:1, :]
        for jj in range(2):
            i = 2 * r + jj
            r0 = pl.multiple_of(i * BL, BL)
            fi = jnp.concatenate([fi_s[0], fi_s[1]], axis=1)
            y = jnp.dot(fi, z_s[slot, i], preferred_element_type=f32)
            y = y + kv_s[ct, pl.ds(r0, BL), :].astype(f32) * dvec
            a = x_s[ct, pl.ds(r0, BL), :].astype(f32) * y
            abg_s[ct, pl.ds(r0, BL), :] = a.astype(bf16)

    NPIECE = D // RP

    def transpose4(v):
        sub = lax.broadcasted_iota(jnp.int32, (8, 128), 0)
        v = list(v)
        for s in (2, 1):
            keep = (sub & s) == 0
            for q in range(4):
                if not q & s:
                    a, b = v[q], v[q + s]
                    v[q] = jnp.where(keep, a, pltpu.roll(b, s, 0))
                    v[q + s] = jnp.where(keep, pltpu.roll(a, 8 - s, 0), b)
        return v

    def relayout(par, half, slot, p):
        def two_tiles(d):
            t = jnp.stack([stage[slot, d], stage[slot, d + RP // 2]])
            return pltpu.bitcast(t.reshape(2 * HC, 128), u32)

        lo, hi = [], []
        for q in range(4):
            ev = two_tiles(p * RP + 2 * q)
            od = two_tiles(p * RP + 2 * q + 1)
            lo.append((ev & jnp.uint32(0xFFFF)) | (od << 16))
            hi.append((ev >> 16) | (od & jnp.uint32(0xFFFF0000)))
        lo = transpose4(lo)
        hi = transpose4(hi)
        r0 = p * (RP // 2)
        rows = pl.ds(r0 if isinstance(p, int) else pl.multiple_of(r0, RP // 2), RP // 2)
        for j in range(HC // 2):
            w_bufs[par][half * HC + 2 * j, rows, :] = lo[j]
            w_bufs[par][half * HC + 2 * j + 1, rows, :] = hi[j]

    def wtile(m, h):
        par, t = tile_of(m, h)
        return pltpu.bitcast(w_bufs[par][t], bf16)

    def bulk_dot(par, half, hh):
        xb = jnp.concatenate(
            [pltpu.bitcast(xb_s[t], bf16) for t in range(NC)], axis=1)
        w = pltpu.bitcast(w_bufs[par][half * HC + hh], bf16)
        r = jnp.dot(xb, w, preferred_element_type=f32).astype(bf16)
        qkv_rings[par][half * HC + hh, 0:BULK // 2, :] = pltpu.bitcast(r, u32)
        return r

    def start_copies(cond):
        def start(pred, make):
            def go():
                for c in make():
                    c.start()
            if pred is True:
                go()
            elif pred is not False:
                pl.when(pred)(go)

        for c in range(NCH - NSLOT):
            start(cond(c), lambda: [w_copy(c + NSLOT, c % NSLOT)])
        for n in range(NC):
            start(cond(n + 1), lambda: [wo_copy(n)])
        for gi, group in enumerate(pre_groups):
            start(cond(gi + 2), lambda: group)

    def chunk_dots(par, half, aslot, nhalf, nslot, first, wot=None):
        for hh in range(HC):
            if hh == first and first > 0:
                w_copy(0, nslot).wait()
            r = bulk_dot(par, half, hh)
            if hh >= first:
                p0 = (hh - first) * NPIECE // (HC - first)
                p1 = (hh - first + 1) * NPIECE // (HC - first)
                for p in range(p0, p1):
                    q0 = ((p - p0) * (BULK // HC) // (p1 - p0)) * HC
                    stage[aslot, D] = r[q0:q0 + HC]
                    relayout(1 - par, nhalf, nslot, p)
                    if wot is not None:
                        wr = H * DH // NPIECE
                        wo_s[aslot, H * DH:H * DH + 8, :] = r[q0:q0 + 8]
                        wo_u[wot, p * wr // 2:(p + 1) * wr // 2, :] = pltpu.bitcast(
                            wo_s[wot, p * wr:(p + 1) * wr, :], u32)

    w_copy(0, 0).wait()
    w_copy(2, 2).start()

    def relayout0(i, carry):
        for q in range(8):
            relayout(0, 0, 0, i * 8 + q)
        return carry

    lax.fori_loop(0, NPIECE // 8, relayout0, 0)
    for n in range(NC):
        x0_copy(n).wait()
        if n == 0:
            w_copy(3, 3).start()
        xb_s[n] = pltpu.bitcast(x_s[n, 0:BULK, :], u32)
    start_copies(lambda c: c == 0)
    chunk_dots(0, 0, zero, 0, 1, 4)

    def pre_body(k, carry):
        for par in (1, 0):
            i = 2 * k + 2 - par
            nslot = (i + 1) % NSLOT
            w_copy(0, nslot).wait()
            start_copies(lambda c: (i == c) if (c % 2 == par and c > 0) else False)

            @pl.when(i >= 3)
            def _():
                wo_copy(i - 3, 0).wait()

            chunk_dots(par, k + 1 - par, i % NSLOT, k + 1, nslot, 0,
                       jnp.where(i >= 3, i - 3, NC))
        return carry

    lax.fori_loop(0, NCH // 2 - 1, pre_body, 0)

    for group in conv_groups:
        for c in group:
            c.wait()
    for c in late:
        c.start()
    taps = shift_s[0].astype(f32)
    dv = dvec_s[0].astype(f32)
    gw = gate_s[0].astype(f32)
    for n in range(NC):
        for tau in range(KS):
            prm_s[n, tau] = jnp.broadcast_to(
                taps[tau:tau + 1, n * 128:(n + 1) * 128], (8, 128))
        prm_s[n, KS] = jnp.broadcast_to(dv[n:n + 1], (8, 128))
        prm_s[n, KS + 1] = jnp.broadcast_to(gw[n:n + 1], (8, 128))

    zpos = pl.multiple_of(zero * 8, 8)
    todo = [(0, KVP * q) for q in range(S // KVP)] + [(1, KVP * q) for q in range(8)]
    per_dot = -(-len(todo) // (HC - 1))
    kv_done = dft_done = 0
    for hh in range(HC):
        r = bulk_dot(1, NCH // 2 - 1, hh)
        ready = min(kv_done * KVP // BL, NB)
        for q, (ct0, row0) in enumerate(todo[kv_done:kv_done + per_dot]):
            kv_anchor(zpos, r[q * 40:q * 40 + 8])
            conv_kv(ct0, row0)
        kv_done = min(kv_done + per_dot, len(todo))
        for d in (2 * hh, 2 * hh + 1):
            conv_filter_dft(0, d, 0)
        for j in range(dft_done, ready):
            conv_kv_dft(0, j, 0)
        dft_done = ready
    assert dft_done == NB
    for group in main_groups:
        for c in group:
            c.wait()

    def attn_mask():
        row = lax.broadcasted_iota(jnp.int32, (2 * LTOT, 2 * LTOT), 0)
        col = lax.broadcasted_iota(jnp.int32, (2 * LTOT, 2 * LTOT), 1)
        row_mem = row >= 2 * SEG
        col_mem = col >= 2 * SEG
        row_head = jnp.where(row_mem, (row - 2 * SEG) // M, row // SEG)
        col_head = jnp.where(col_mem, (col - 2 * SEG) // M, col // SEG)
        same = row_head == col_head
        mask = same & (row_mem | col_mem | (col <= row))
        fill = jnp.where(same, -1e9 / scale, -jnp.inf).astype(f32)
        return mask, fill

    def step(s, mem, do_fwd, odd):
        mask, fill = attn_mask()

        ct = s >> 3
        r = s & 7
        cnext = jnp.minimum(ct + 1, NC - 1)
        cprev = jnp.maximum(ct - 1, 0)
        slot = ct & 1
        oslot = 1 - slot

        o16, o8 = (8, 0) if odd else (0, 16)
        al = 8 if odd is None else 16

        def pieces(base, wrap):
            f = _ring if wrap else (lambda v: v)
            if odd is None:
                return [(pl.multiple_of(f(base + 8 * j), 8), 8) for j in range(3)]
            return [(pl.multiple_of(f(base + o16), 16), 16),
                    (pl.multiple_of(f(base + o8), 8), 8)]

        xpos = pieces(BULK + TP * s, False)
        wpos = pieces(BULK + TP * s, True)
        bpos = pieces(TP * s, False)
        rpos = pl.multiple_of(_ring(SEG * s), SEG)
        l16 = pl.multiple_of(_ring(TP * s + o16), al)
        l8 = pl.multiple_of(_ring(TP * s + o8), 8)

        def store_rows(ref, lead, pos, val):
            r0 = 0
            for p0, n in pos:
                ref[lead, pl.ds(p0, n), :] = val[r0:r0 + n]
                r0 += n

        rhalf = pl.multiple_of(rpos >> 1, SEG // 2)
        gpos = pl.multiple_of(SEG * s, SEG)
        apos = pl.multiple_of(r * 8, 8)
        kpos = pl.multiple_of((r & 1) * 8, 8)

        lhs = jnp.concatenate(
            [jnp.concatenate([x_s[t, pl.ds(p0, n), :] for t in range(NC)], axis=1)
             for p0, n in xpos] + [mem], axis=0)

        rls = [None] * H
        acc = [None] * NC

        prods = conv_products(r, slot)
        ckv = jnp.minimum(((s + 1) >> 3) + 1, NC - 1)
        kv_rows = [pl.multiple_of(((s + 1) & 7) * 2 * BL + q * KVP, KVP)
                   for q in range(2 * BL // KVP)] if do_fwd else []

        def release(key, res):
            n_prod, n_kv = PLAN.get(key, (0, 0))
            if n_prod:
                uk_s[4 * NB, pl.ds(apos, 8), :] = res[0:8]
                for _ in range(n_prod):
                    next(prods, None)
            if n_kv and kv_rows:
                kv_anchor(kpos, res[0:8].astype(bf16))
                conv_kv(ckv, kv_rows.pop(0))

        n_dot = [0]

        def proj(m, h):
            ri, t = tile_of(m, h)
            res = jnp.dot(lhs, wtile(m, h), preferred_element_type=f32)
            release(n_dot[0], res)
            n_dot[0] += 1
            res = res.astype(bf16)
            r0 = 0
            for p0, n in wpos:
                qkv_rings[ri][t, pl.ds(pl.multiple_of(p0 >> 1, n // 2), n // 2), :] = (
                    pltpu.bitcast(res[r0:r0 + n], u32))
                r0 += n
            qm_s[m * (H // 2) + h // 2, (h % 2) * M:(h % 2 + 1) * M, :] = res[TP:]

        def pair_rows(m, h):
            ri, t = tile_of(m, h)
            tok = [pltpu.bitcast(qkv_rings[ri][t + i, pl.ds(rhalf, SEG // 2), :], bf16)
                   for i in range(2)]
            return jnp.concatenate(tok + [qm_s[m * (H // 2) + h // 2]], axis=0)

        def att_qk(h):
            sc = lax.dot_general(pair_rows(0, h), pair_rows(1, h),
                                 (((1,), (1,)), ((), ())), preferred_element_type=f32)
            sc = jnp.where(mask, sc, fill)
            mx = jnp.max(sc, axis=-1, keepdims=True)
            p = jnp.exp2((sc - mx) * (scale * math.log2(math.e)))
            den = jnp.sum(p, axis=-1, keepdims=True)
            rl = pl.reciprocal(den, approx=True)
            rls[h] = rl * (2.0 - den * rl)
            p_s[h // 2] = p.astype(bf16)

        def att_pv(h):
            ri, t = ring_of(h)
            o = jnp.dot(p_s[h // 2], pair_rows(2, h), preferred_element_type=f32)
            o = (o * rls[h]).astype(bf16)
            for i in range(2):
                o_rings[ri][t + i, pl.ds(rpos, SEG), :] = o[i * SEG:(i + 1) * SEG]
            for i in range(2):
                l2_s[h + i, M:, :] = o[2 * SEG + i * M:2 * SEG + (i + 1) * M]
            for i in range(2):
                l2_s[h + i, 0:M, :] = o_rings[ri][t + i, pl.ds(l8, M), :]

        def wo_grp(g):
            h0 = g * G
            parts = []
            for h in range(h0, h0 + G):
                ri, t = ring_of(h)
                parts.append(jnp.concatenate(
                    [o_rings[ri][t, pl.ds(l16, 16), :], l2_s[h]], axis=0))
            l2 = jnp.concatenate(parts, axis=1)
            for n in range(NC):
                w = pltpu.bitcast(wo_u[n, h0 * DH // 2:(h0 + G) * DH // 2, :], bf16)
                res = jnp.dot(l2, w, preferred_element_type=f32)
                if g == 0:
                    acc_s[n] = res
                else:
                    acc[n] = (acc_s[n] if g == 1 else acc[n]) + res

        def gate():
            tot = None
            for n in range(NC):
                xv = x_s[n, pl.ds(gpos, SEG), :].astype(f32) * prm_s[n, KS + 1, 0:1, :]
                tot = xv if tot is None else tot + xv
            z = jnp.sum(tot, axis=-1, keepdims=True)
            abg_s[2 * NC, pl.ds(gpos, SEG), :] = jnp.broadcast_to(
                jax.nn.sigmoid(z), (SEG, 128)).astype(bf16)

        def qkv_grp(g):
            heads = range(g * G, (g + 1) * G)
            for h in heads:
                proj(2, h)
            for h in heads:
                proj(0, h)
                proj(1, h)

        def qk_grp(g):
            for h in range(g * G, (g + 1) * G, 2):
                att_qk(h)

        def pv_grp(g):
            for h in range(g * G, (g + 1) * G, 2):
                att_pv(h)

        conv_inverse(cprev, r, oslot)
        if do_fwd:
            for jj in range(2):
                conv_filter_dft(cnext, 2 * r + jj, oslot)
            for jj in range(2):
                conv_kv_dft(cnext, 2 * r + jj, oslot)
        qkv_grp(0)
        qkv_grp(1)
        qk_grp(0)
        qkv_grp(2)
        pv_grp(0)
        qk_grp(1)
        qkv_grp(3)
        gate()
        pv_grp(1)
        qk_grp(2)
        wo_grp(0)
        pv_grp(2)
        qk_grp(3)
        wo_grp(1)
        pv_grp(3)
        wo_grp(2)
        wo_grp(3)
        for _ in prods:
            pass
        assert not kv_rows
        new_mem = []
        for n in range(NC):
            res = acc[n].astype(bf16)
            store_rows(abg_s, NC + n, bpos, res)
            new_mem.append(res[TP:])
        return jnp.concatenate(new_mem, axis=1)

    def step_pair(it, carry):
        @pl.when(it == 3)
        def _():
            late_all.wait()

        mem = step(2 * it, mem_s[...], True, 0)
        mem_s[...] = step(2 * it + 1, mem, True, 1)
        return carry

    def step_last(s, carry):
        mem_s[...] = step(s, mem_s[...], False, None)
        return carry

    lax.fori_loop(0, (NSEG - NLAST) // 2, step_pair, 0)
    lax.fori_loop(NSEG - NLAST, NSEG, step_last, 0)

    q0 = P0 % RING

    TB = 64
    HB = 64
    KP = 4

    def combine(n, rows, b):
        g = abg_s[2 * NC + zero, rows, :].astype(f32)
        a = abg_s[n + zero, rows, :].astype(f32)
        if b is None:
            b = abg_s[NC + n + zero, rows, :]
        b = b.astype(f32)
        abg_s[NC + n, rows, :] = (g * a + (1.0 - g) * b).astype(bf16)

    def post_tile(n):
        conv_inverse(NC - 1, n, (NC - 1) & 1)
        piece = 0
        for c in range(BULK // TB):
            r0 = (q0 + c * TB) % RING
            tail = None
            for kp in range(KP):
                hs = range(kp * H // KP, (kp + 1) * H // KP)
                l2 = jnp.concatenate(
                    [o_rings[ring_of(h)[0]][ring_of(h)[1], r0:r0 + TB, :] for h in hs],
                    axis=1)
                w = wo_u[n, hs[0] * DH // 2:(hs[-1] + 1) * DH // 2, :]
                res = jnp.dot(l2, pltpu.bitcast(w, bf16), preferred_element_type=f32)
                tail = res if tail is None else tail + res
                if kp == KP - 1:
                    combine(n, slice(P0 + c * TB, P0 + (c + 1) * TB), tail.astype(bf16))
                elif piece < P0 // HB:
                    abg_s[2 * NC + 1, 0:16, :] = tail[0:16].astype(bf16)
                if piece < P0 // HB:
                    combine(n, slice(piece * HB, (piece + 1) * HB), None)
                    piece += 1
                    if piece == P0 // HB:
                        out_copy(n, 0).start()
        out_copy(n, 1).start()

    def post_body(it, carry):
        post_tile(2 * it)
        post_tile(2 * it + 1)
        return carry

    lax.fori_loop(0, NC // 2, post_body, 0)
    for n in range(NC):
        out_copy(n, 0).wait()
        out_copy(n, 1).wait()


@jax.jit
def pallas_gated_mix__ssm_conv_h3__memory_aug_recurrent_mem_tr__prompt_kernel(
    A_q: jax.Array,
    A_k: jax.Array,
    A_v: jax.Array,
    A_shift_k: jax.Array,
    A_ssm_k: jax.Array,
    A_ssm_D: jax.Array,
    B_x: jax.Array,
    B_mem0: jax.Array,
    B_Wq: jax.Array,
    B_Wk: jax.Array,
    B_Wv: jax.Array,
    B_Wo: jax.Array,
    B_seg_len,
    gate_w: jax.Array,
):
    del B_x
    del B_seg_len
    assert A_q.shape == (1, S, D) and B_Wq.shape == (D, H, DH)
    assert B_mem0.shape == (1, M, D) and A_shift_k.shape == (D, KS)

    n_pre = NB + 4 + 4 + NC
    scratch = [
        pltpu.VMEM((NC, S, 128), bf16),
        pltpu.VMEM((NC, BULK // 2, 128), u32),
        pltpu.VMEM((2, NC, S + 2 * PAD, 128), bf16),
        pltpu.VMEM((NB, D, 128), bf16),
        pltpu.VMEM((NC, S, 128), bf16),
        pltpu.VMEM((2 * NC + 2, S, 128), bf16),
        pltpu.VMEM((3 * H // 2, D // 2, 128), u32),
        pltpu.VMEM((3 * H // 2, D // 2, 128), u32),
        pltpu.VMEM((NC + 1, H * DH + 64, 128), bf16),
        pltpu.VMEM((NC + 1, H * DH // 2, 128), u32),
        pltpu.VMEM((NSLOT, D + 8, HC, 128), bf16),
        pltpu.VMEM((3 * H // 2, RING // 2, 128), u32),
        pltpu.VMEM((3 * H // 2, RING // 2, 128), u32),
        pltpu.VMEM((H // 2, RING, 128), bf16),
        pltpu.VMEM((H // 2, RING, 128), bf16),
        pltpu.VMEM((4 * NB + 1, NF, 128), f32),
        pltpu.VMEM((2, NB, NF, 128), bf16),
        pltpu.VMEM((NF, BL), bf16),
        pltpu.VMEM((2, BL, BL), bf16),
        pltpu.VMEM((H // 2, 2 * LTOT, 2 * LTOT), bf16),
        pltpu.VMEM((NC, TP + M, 128), f32),
        pltpu.VMEM((3 * H // 2, 2 * M, 128), bf16),
        pltpu.VMEM((H, 2 * M, 128), bf16),
        pltpu.VMEM((M, D), bf16),
        pltpu.VMEM((2, KS, D), bf16),
        pltpu.VMEM((8, NC, 128), bf16),
        pltpu.VMEM((8, NC, 128), bf16),
        pltpu.VMEM((NC, KS + 2, 8, 128), f32),
        pltpu.SMEM((1,), jnp.int32),
        pltpu.SemaphoreType.DMA((NSLOT,)),
        pltpu.SemaphoreType.DMA((NC,)),
        pltpu.SemaphoreType.DMA((NC,)),
        pltpu.SemaphoreType.DMA((n_pre,)),
        pltpu.SemaphoreType.DMA((1,)),
        pltpu.SemaphoreType.DMA((2 * NC,)),
    ]
    out = pl.pallas_call(
        _kernel,
        out_shape=jax.ShapeDtypeStruct((S, D), bf16),
        in_specs=[pl.BlockSpec(memory_space=pl.ANY)] * 12,
        out_specs=pl.BlockSpec(memory_space=pl.ANY),
        scratch_shapes=scratch,
        compiler_params=pltpu.CompilerParams(
            vmem_limit_bytes=124 * 1024 * 1024,
            disable_bounds_checks=True,
            disable_semaphore_checks=True),
    )(
        A_q.reshape(S, D), A_k.reshape(S, D), A_v.reshape(S, D),
        A_shift_k.T, A_ssm_k, A_ssm_D.reshape(NC, 128), B_mem0.reshape(M, D),
        B_Wq, B_Wk, B_Wv, B_Wo.reshape(H * DH, D), gate_w.reshape(NC, 128),
    )
    return out.reshape(1, S, D)
```
